```python
import jax
import jax.numpy as jnp

def _softmax(x, axis=-1):
    return jax.nn.softmax(x, axis=axis)
def _gelu(x):
    return jax.nn.gelu(x, approximate=True)
def _silu(x):
    return jax.nn.silu(x)
def _sigmoid(x):
    return jax.nn.sigmoid(x)
def _layernorm(x, axis=-1, eps=1e-5):
    m = jnp.mean(x, axis=axis, keepdims=True)
    v = jnp.var(x, axis=axis, keepdims=True)
    return (x - m) / jnp.sqrt(v + eps)
def _scatter_add(tgt, idx, src, axis=0):
    return tgt.at[idx].add(src)
def _segment_sum(src, seg, n):
    return jax.ops.segment_sum(src, seg, n)
class _Rng:
    def __init__(self, key):
        self._k = key
    def _next(self):
        self._k, sub = jax.random.split(self._k)
        return sub
    def normal(self, shape):
        return jax.random.normal(self._next(), shape, dtype=jnp.bfloat16)
    def randint(self, lo, hi, shape):
        return jax.random.randint(self._next(), shape, lo, hi, dtype=jnp.int32)
    def uniform(self, shape, lo=0.0, hi=1.0):
        return jax.random.uniform(self._next(), shape, jnp.bfloat16, lo, hi)
    def permutation(self, n):
        return jax.random.permutation(self._next(), n)


kernel_name = 'gated_mix__linear_attn_block__moe_arch_mod__prompt'

def setup_inputs():
    _rng = _Rng(jax.random.key(int.from_bytes(__import__("os").urandom(4), "little")))
    _w = (lambda a: (lambda t: t.astype(jnp.bfloat16) if jnp.issubdtype(t.dtype, jnp.floating) else t)(jnp.asarray(a)))
    def _A_setup():
        B, S, D = 1, 2048, 1024
        return {
            "x": _w((lambda *s: _rng.normal(s) * 0.05)(B, S, D)),
            "wqkv": _w((lambda *s: _rng.normal(s) * 0.05)(D, 3 * D)),
            "wo": _w((lambda *s: _rng.normal(s) * 0.05)(D, D)),
        }
    _A_in = _A_setup()

    def _B_setup():
        B, S, D, F, C = 1, 2048, 1024, 3584, 1
        return {
            "x": _w((lambda *s: _rng.normal(s) * 0.05)(B, S, D)),
            "w_r": _w((lambda *s: _rng.normal(s) * 0.05)(D)),
            "w_gate": _w((lambda *s: _rng.normal(s) * 0.05)(D, F)),
            "w_up": _w((lambda *s: _rng.normal(s) * 0.05)(D, F)),
            "w_down": _w((lambda *s: _rng.normal(s) * 0.05)(F, D)),
        }
    _B_in = _B_setup()

    return {
        "A_x": _A_in["x"],
        "A_wqkv": _A_in["wqkv"],
        "A_wo": _A_in["wo"],
        "B_x": _B_in["x"],
        "B_w_r": _B_in["w_r"],
        "B_w_gate": _B_in["w_gate"],
        "B_w_up": _B_in["w_up"],
        "B_w_down": _B_in["w_down"],
        "gate_w": _w((lambda *s: _rng.normal(s) * 0.05)(1024)),
    }

def reference(A_x, A_wqkv, A_wo, B_x, B_w_r, B_w_gate, B_w_up, B_w_down, gate_w):
    def _A_ref(x, wqkv, wo):
        B, S, D = x.shape
        H = 32; Dh = D // H
        qkv = (lambda x, *d: x.transpose(*d))((x @ wqkv).reshape(B, S, 3, H, Dh), 2, 0, 3, 1, 4)
        q, k, v = qkv[0], qkv[1], qkv[2]
        phi = lambda t: jnp.where(t > 0, t + 1, jnp.exp(t)) + 1e-6
        pq, pk = phi(q), phi(k)
        kv = jnp.einsum("bhsd,bhse->bhde", pk, v)
        z = jnp.einsum("bhsd->bhd", pk)
        num = jnp.einsum("bhqd,bhde->bhqe", pq, kv)
        den = jnp.einsum("bhqd,bhd->bhq", pq, z)[..., None] + 1e-6
        o = num / den
        return (lambda x, *d: x.transpose(*d))(o, 0, 2, 1, 3).reshape(B, S, D) @ wo

    def _B_ref(x, w_r, w_gate, w_up, w_down):
        B, S, D = x.shape
        C = 1
        r = x @ w_r
        idx = jnp.argsort(-r, axis=-1)[:, :C]
        idx_e = jnp.repeat(idx.reshape(B, C, 1), D, axis=2)
        x_sel = jnp.take_along_axis(x, idx_e, axis=1)
        g = _silu(x_sel @ w_gate)
        u = x_sel @ w_up
        y = (g * u) @ w_down
        r_sel = _sigmoid(jnp.take_along_axis(r, idx, axis=1))
        y = y * r_sel.reshape(B, C, 1)
        b_off = (jnp.arange(B) * S).reshape(B, 1)
        flat_idx = (idx + b_off).reshape(B * C)
        zero = (x * 0.0).reshape(B * S, D)
        upd = _scatter_add(zero, flat_idx, y.reshape(B * C, D), axis=0)
        return x + upd.reshape(B, S, D)

    x = A_x
    g = _sigmoid((x * gate_w).sum(-1, keepdims=True))
    a = _A_ref(x, A_wqkv, A_wo)
    b = _B_ref(x, B_w_r, B_w_gate, B_w_up, B_w_down)
    return g * a + (1 - g) * b
```

```python
import jax
import jax.numpy as jnp
from jax import lax
import jax.experimental.pallas as pl
import jax.experimental.pallas.tpu as pltpu

S = 2048
D = 1024
F = 3584
H = 32
DH = D // H
T = 512
NT_ = S // T
BLK = 128
NB = D // BLK

_NT = (((1,), (1,)), ((), ()))
_TN = (((0,), (0,)), ((), ()))
f32 = jnp.float32
bf16 = jnp.bfloat16


def _phi(t):
    return jnp.where(t > 0, t + 1.0, jnp.exp(t)) + 1e-6


def _sigmoid(t):
    return 1.0 / (1.0 + jnp.exp(-t))


def _kernel(x_hbm, wqkv_hbm, wo_hbm, wr_ref, wg_hbm, wu_hbm, wd_hbm, gw_ref,
            out_hbm,
            x_v, wq_v, wk_v, wv_v, wo_v, wg_v, wu_v, wd_v,
            pkT_v, wqT_v, g_v, m_v, pT_v, out_v, gate_v, zc_v, y_v,
            sem_x, sem_w, sem_o):
    def x_copy(i):
        return pltpu.make_async_copy(x_hbm.at[0, pl.ds(i * T, T), :],
                                     x_v.at[pl.ds(i * T, T), :], sem_x.at[i])

    cp_wk = pltpu.make_async_copy(wqkv_hbm.at[:, pl.ds(D, D)], wk_v, sem_w.at[0])
    cp_wq = pltpu.make_async_copy(wqkv_hbm.at[:, pl.ds(0, D)], wq_v, sem_w.at[1])
    cp_wv = pltpu.make_async_copy(wqkv_hbm.at[:, pl.ds(2 * D, D)], wv_v, sem_w.at[2])
    cp_wo = pltpu.make_async_copy(wo_hbm, wo_v, sem_w.at[3])
    cp_wg = pltpu.make_async_copy(wg_hbm, wg_v, sem_w.at[4])
    cp_wu = pltpu.make_async_copy(wu_hbm, wu_v, sem_w.at[5])
    cp_wd = pltpu.make_async_copy(wd_hbm, wd_v, sem_w.at[6])

    def out_copy(i):
        return pltpu.make_async_copy(out_v.at[pl.ds(i * T, T), :],
                                     out_hbm.at[0, pl.ds(i * T, T), :], sem_o.at[i])

    x_copy(0).start()
    cp_wk.start()
    for i in range(1, NT_):
        x_copy(i).start()
    cp_wq.start(priority=1)
    cp_wv.start(priority=1)
    cp_wo.start(priority=1)
    cp_wg.start(priority=1)
    cp_wu.start(priority=1)
    cp_wd.start(priority=1)

    wr = wr_ref[...].astype(f32)
    gw = gw_ref[...].astype(f32)

    cp_wk.wait()
    zacc = jnp.zeros((8, D), f32)
    best_v = jnp.full((1, 1), -jnp.inf, f32)
    best_i = jnp.zeros((1, 1), jnp.int32)
    for i in range(NT_):
        x_copy(i).wait()
        xt = x_v[pl.ds(i * T, T), :]
        k = jnp.dot(xt, wk_v[...], preferred_element_type=f32)
        pk = _phi(k)
        zacc = zacc + jnp.sum(pk.reshape(T // 8, 8, D), axis=0)
        pkT_v[:, pl.ds(i * T, T)] = pk.astype(bf16).T
        xf = xt.astype(f32)
        gl = jnp.sum(xf * gw, axis=1, keepdims=True)
        gate_v[pl.ds(i * T, T), :] = jnp.broadcast_to(_sigmoid(gl), (T, BLK))
        r = jnp.sum(xf * wr, axis=1, keepdims=True).astype(bf16).astype(f32)
        m = jnp.max(r, axis=0, keepdims=True)
        rows = lax.broadcasted_iota(jnp.int32, (T, 1), 0) + i * T
        mi = jnp.min(jnp.where(r == m, rows, S), axis=0, keepdims=True)
        take = m > best_v
        best_i = jnp.where(take, mi, best_i)
        best_v = jnp.where(take, m, best_v)

    z = jnp.sum(zacc, axis=0, keepdims=True)
    zc_v[...] = jnp.broadcast_to(z, (BLK, D)).T
    idx = jnp.clip(best_i[0, 0], 0, S - 1)

    for j in range(2):
        rows = pl.ds(j * 512, 512)
        g_v[rows, :] = jnp.dot(pkT_v[rows, :], x_v[...],
                               preferred_element_type=f32).astype(bf16)

    cp_wv.wait()
    cp_wo.wait()
    cp_wq.wait()
    ri = lax.broadcasted_iota(jnp.int32, (BLK, BLK), 0) // DH
    ci = lax.broadcasted_iota(jnp.int32, (BLK, BLK), 1) // DH
    diag = ri == ci
    for j in range(NB):
        sl = pl.ds(j * BLK, BLK)
        kv = jnp.dot(g_v[sl, :], wv_v[:, sl], preferred_element_type=f32)
        kv = jnp.where(diag, kv, 0.0).astype(bf16)
        m_v[sl, :] = jnp.dot(kv, wo_v[sl, :], preferred_element_type=f32).astype(bf16)
    wqT_v[...] = wq_v[...].T

    for i in range(NT_):
        qT = lax.dot_general(wqT_v[...], x_v[pl.ds(i * T, T), :], _NT,
                             preferred_element_type=f32)
        pq = _phi(qT)
        zc = jnp.tile(zc_v[...], (1, T // BLK))
        den = jnp.sum((pq * zc).reshape(H, DH, T), axis=1, keepdims=True) + 1e-6
        p = pq.reshape(H, DH, T) * (1.0 / den)
        pT_v[:, pl.ds(i * T, T)] = p.reshape(D, T).astype(bf16)

    cp_wg.wait()
    cp_wu.wait()
    cp_wd.wait()
    base = pl.multiple_of((idx // 16) * 16, 16)
    xs = x_v[pl.ds(base, 16), :]
    gg = jnp.dot(xs, wg_v[...], preferred_element_type=f32)
    uu = jnp.dot(xs, wu_v[...], preferred_element_type=f32)
    hh = (gg * _sigmoid(gg) * uu).astype(bf16)
    yy = jnp.dot(hh, wd_v[...], preferred_element_type=f32)
    sel = lax.broadcasted_iota(jnp.int32, (16, D), 0) == (idx - base)
    y = jnp.sum(jnp.where(sel, yy, 0.0), axis=0, keepdims=True) * _sigmoid(best_v)
    y_v[...] = jnp.broadcast_to(y, (8, D))

    for i in range(NT_):
        a = lax.dot_general(pT_v[:, pl.ds(i * T, T)], m_v[...], _TN,
                            preferred_element_type=f32)
        g = jnp.tile(gate_v[pl.ds(i * T, T), :], (1, NB))
        rows = lax.broadcasted_iota(jnp.int32, (T, D), 0) + i * T
        upd = jnp.where(rows == idx, y_v[0:1, :], 0.0)
        b = x_v[pl.ds(i * T, T), :].astype(f32) + upd
        out_v[pl.ds(i * T, T), :] = (g * a + (1.0 - g) * b).astype(bf16)
        out_copy(i).start()
    for i in range(NT_):
        out_copy(i).wait()


@jax.jit
def pallas_gated_mix__linear_attn_block__moe_arch_mod__prompt_kernel(
    A_x: jax.Array,
    A_wqkv: jax.Array,
    A_wo: jax.Array,
    B_x: jax.Array,
    B_w_r: jax.Array,
    B_w_gate: jax.Array,
    B_w_up: jax.Array,
    B_w_down: jax.Array,
    gate_w: jax.Array,
):
    del B_x
    any_spec = pl.BlockSpec(memory_space=pl.ANY)
    vmem_spec = pl.BlockSpec(memory_space=pltpu.VMEM)
    scratch = [
        pltpu.VMEM((S, D), bf16),
        pltpu.VMEM((D, D), bf16),
        pltpu.VMEM((D, D), bf16),
        pltpu.VMEM((D, D), bf16),
        pltpu.VMEM((D, D), bf16),
        pltpu.VMEM((D, F), bf16),
        pltpu.VMEM((D, F), bf16),
        pltpu.VMEM((F, D), bf16),
        pltpu.VMEM((D, S), bf16),
        pltpu.VMEM((D, D), bf16),
        pltpu.VMEM((D, D), bf16),
        pltpu.VMEM((D, D), bf16),
        pltpu.VMEM((D, S), bf16),
        pltpu.VMEM((S, D), bf16),
        pltpu.VMEM((S, BLK), f32),
        pltpu.VMEM((D, BLK), f32),
        pltpu.VMEM((8, D), f32),
        pltpu.SemaphoreType.DMA((NT_,)),
        pltpu.SemaphoreType.DMA((7,)),
        pltpu.SemaphoreType.DMA((NT_,)),
    ]
    return pl.pallas_call(
        _kernel,
        out_shape=jax.ShapeDtypeStruct((1, S, D), bf16),
        in_specs=[any_spec, any_spec, any_spec, vmem_spec, any_spec, any_spec,
                  any_spec, vmem_spec],
        out_specs=any_spec,
        scratch_shapes=scratch,
        compiler_params=pltpu.CompilerParams(vmem_limit_bytes=110 * 1024 * 1024),
    )(A_x, A_wqkv, A_wo, B_w_r.reshape(1, D), B_w_gate, B_w_up, B_w_down,
      gate_w.reshape(1, D))
```

```python
import os
import jax
import jax.numpy as jnp
from jax import lax
import jax.experimental.pallas as pl
import jax.experimental.pallas.tpu as pltpu

S = 2048
D = 1024
F = 3584
H = 32
DH = D // H
HS = S // 2
HD = D // 2
R = 256
NP = HS // R
BLK = 128
NB = D // BLK
WC = 256

SCOPES = os.environ.get("K_SCOPES", "0") == "1"

_NN = (((1,), (0,)), ((), ()))
_NT = (((1,), (1,)), ((), ()))
_TN = (((0,), (0,)), ((), ()))
f32 = jnp.float32
bf16 = jnp.bfloat16

A_PIECES = ((0, 256), (256, 256), (512, 256), (768, 128), (896, 128))

A_FORM = (0, 1, 5, 6, 2, 3, 4)
B_FORM = (0, 5, 4, 3, 6, 2, 1)


def _forms(b11, b12, b21, b22):
    return (b11 + b22, b21 + b22, b11 + b12, b21 - b11, b12 - b22, b11, b22)


def _strassen(prod):
    m3 = prod(2)
    m4 = prod(3)
    m5 = prod(4)
    c12 = m3 + m5
    m2 = prod(1)
    c21 = m2 + m4
    m1 = prod(0)
    m7 = prod(6)
    c11 = (m1 + m4) + (m7 - m5)
    m6 = prod(5)
    c22 = (m1 - m2) + (m3 + m6)
    return c11, c12, c21, c22


def _strassen_head(prod):
    m3 = prod(2)
    m4 = prod(3)
    m5 = prod(4)
    c12 = m3 + m5
    m2 = prod(1)
    c21 = m2 + m4
    m1 = prod(0)
    return c12, c21, (m1 + m4) - m5, (m1 - m2) + m3


def _strassen_tail(prod, head):
    c12, c21, t11, t22 = head
    c11 = t11 + prod(6)
    c22 = t22 + prod(5)
    return c11, c12, c21, c22


def _chained_forms(blocks, live, prev, slow):
    halves = []
    for h in range(2):
        b11, b12, b21, b22 = (b[:, BLK * h:BLK * (h + 1)] for b in blocks)
        link = jnp.where(live, 0.0, prev)
        b11 = b11 + link
        s1112 = b11 + b12
        if slow:
            link = jnp.where(live, 0.0, s1112)
        b22 = b22 + link
        prev = b11 + b22
        halves.append((prev, b21 + b22, s1112, b21 - b11, b12 - b22, b11, b22))
    forms = [jnp.concatenate([halves[0][f], halves[1][f]], axis=1).astype(bf16)
             for f in range(7)]
    return forms, prev


def _dot(a, b, dims=_NN):
    return lax.dot_general(a, b, dims, preferred_element_type=f32)


def _phi(t):
    return jnp.where(t > 0, t + 1.0, jnp.exp(t)) + 1e-6


def _sigmoid(t):
    return 1.0 / (1.0 + jnp.exp(-t))


class _Scope:
    def __init__(self, name):
        self.c = jax.named_scope(name) if SCOPES else None
    def __enter__(self):
        if self.c is not None:
            self.c.__enter__()
    def __exit__(self, *a):
        if self.c is not None:
            self.c.__exit__(*a)


def _matvec_chains(w_refs, col_ref, n_rows, n_cols, live):
    live2 = jnp.concatenate([live, live], axis=1)
    outs = [[] for _ in w_refs]
    acc = jnp.zeros((8, 2 * BLK), f32)
    for c0 in range(0, n_cols, 2 * BLK):
        for w_ref, out in zip(w_refs, outs):
            def step(i, acc, w_ref=w_ref):
                r0 = pl.multiple_of(i * 8, 8)
                col = col_ref[pl.ds(r0, 8), :]
                w = w_ref[pl.ds(r0, 8), c0:c0 + 2 * BLK].astype(f32)
                return acc + w * jnp.concatenate([col, col], axis=1)
            acc = lax.fori_loop(0, n_rows // 8, step, jnp.where(live2, 0.0, acc), unroll=True)
            out.append(acc)
    return [jnp.sum(jnp.concatenate(o, axis=1), axis=0, keepdims=True) for o in outs]


def _kernel(x_hbm, wqkv_hbm, wo_hbm, wr_hbm, wg_hbm, wu_hbm, wd_hbm, gw_hbm,
            out_hbm,
            x_v, wq_v, wk_v, wv_v, wo_v, wg_v, wu_v, wd_v, wr_v, gw_v,
            xs_v, wks_v, wqs_v, pks_v, g_v, ms_v, ps_v, out_v,
            gate_v, zc_v, xc_v, hc_v,
            sem_hi, sem_lo, sem_o):
    NK = D // WC

    def x_copy(j, half):
        r0 = half * HS + j * R
        return pltpu.make_async_copy(x_hbm.at[0, pl.ds(r0, R), :],
                                     x_v.at[pl.ds(r0, R), :],
                                     sem_hi.at[NK + 2 * j + half])

    def wk_copy(c):
        return pltpu.make_async_copy(wqkv_hbm.at[:, pl.ds(D + c * WC, WC)],
                                     wk_v.at[:, pl.ds(c * WC, WC)], sem_hi.at[c])

    cp_wq = pltpu.make_async_copy(wqkv_hbm.at[:, pl.ds(0, D)], wq_v, sem_lo.at[0])
    cp_wv = pltpu.make_async_copy(wqkv_hbm.at[:, pl.ds(2 * D, D)], wv_v, sem_lo.at[1])
    cp_wo = pltpu.make_async_copy(wo_hbm, wo_v, sem_lo.at[2])
    cp_wg = pltpu.make_async_copy(wg_hbm, wg_v, sem_lo.at[3])
    cp_wu = pltpu.make_async_copy(wu_hbm, wu_v, sem_lo.at[4])
    cp_wd = pltpu.make_async_copy(wd_hbm, wd_v, sem_lo.at[5])
    cp_wr = pltpu.make_async_copy(wr_hbm, wr_v, sem_lo.at[6])
    cp_gw = pltpu.make_async_copy(gw_hbm, gw_v, sem_lo.at[7])

    def out_copy(i, half, col):
        r0, n = A_PIECES[i]
        r0 = r0 + half * HS
        return pltpu.make_async_copy(out_v.at[pl.ds(r0, n), pl.ds(col * HD, HD)],
                                     out_hbm.at[0, pl.ds(r0, n), pl.ds(col * HD, HD)],
                                     sem_o.at[4 * i + 2 * half + col])

    x_copy(0, 0).start()
    wk_copy(0).start()
    wk_copy(1).start()
    x_copy(0, 1).start()
    wk_copy(2).start()
    wk_copy(3).start()
    for j in range(1, NP):
        x_copy(j, 0).start()
        x_copy(j, 1).start()
    for cp in (cp_wr, cp_gw, cp_wg, cp_wu, cp_wq, cp_wv, cp_wo, cp_wd):
        cp.start(priority=1)

    def x_form(f, r0, n):
        if f == 5:
            return x_v[r0:r0 + n, 0:HD]
        if f == 6:
            return x_v[HS + r0:HS + r0 + n, HD:D]
        return xs_v[f, r0:r0 + n, :]

    def wk_form(f):
        if f == 5:
            return wk_v[0:HD, 0:HD]
        if f == 6:
            return wk_v[HD:D, HD:D]
        return wks_v[f]

    x_copy(0, 0).wait()
    words = pltpu.bitcast(x_v[0:16, 0:BLK], jnp.int32)
    live = lax.shift_right_arithmetic(words, 31) >= -1
    zero = jnp.zeros((8, BLK), f32)

    def ref_forms(src, dst, r0, n, half_rows, slow):
        def step(i, prev):
            r = pl.multiple_of(r0 + i * 8, 8)
            r2 = pl.multiple_of(half_rows + r0 + i * 8, 8)
            for c in range(0, HD, 2 * BLK):
                blocks = [src[pl.ds(rr, 8), cc:cc + 2 * BLK].astype(f32)
                          for rr in (r, r2) for cc in (c, HD + c)]
                fs, prev = _chained_forms(blocks, live, prev, slow)
                for f in range(5):
                    dst[f, pl.ds(r, 8), c:c + 2 * BLK] = fs[f]
            return prev
        lax.fori_loop(0, n // 8, step, zero, unroll=True)

    def make_x_forms(j):
        ref_forms(x_v, xs_v, j * R, R, HS, True)

    def make_wq_forms():
        prev = zero
        for r in range(0, HD, BLK):
            for c in range(0, HD, 2 * BLK):
                tiles = [wq_v[rr:rr + 2 * BLK, cc:cc + BLK].T.astype(f32)
                         for rr, cc in ((c, r), (c, HD + r), (HD + c, r), (HD + c, HD + r))]
                for s0 in range(0, BLK, 8):
                    blocks = [t[s0:s0 + 8] for t in tiles]
                    fs, prev = _chained_forms(blocks, live, prev, True)
                    for f in range(7):
                        wqs_v[f, r + s0:r + s0 + 8, c:c + 2 * BLK] = fs[f]

    zacc = [jnp.zeros((8, HD), f32), jnp.zeros((8, HD), f32)]

    def k_epi(j, c):
        p11, p12, p21, p22 = (_phi(t) for t in c)
        zacc[0] = zacc[0] + jnp.sum((p11 + p21).reshape(R // 8, 8, HD), axis=0)
        zacc[1] = zacc[1] + jnp.sum((p12 + p22).reshape(R // 8, 8, HD), axis=0)
        fs = _forms(p11, p21, p12, p22)
        for f in range(7):
            pks_v[f, :, j * R:(j + 1) * R] = fs[f].astype(bf16).T

    def k_prod(j):
        return lambda i: _dot(x_form(A_FORM[i], j * R, R), wk_form(B_FORM[i]))

    rid = lax.broadcasted_iota(jnp.int32, (16, D), 0)

    with _Scope("ramp"):
        wk_copy(0).wait()
        u0 = _dot(x_v[0:R, :], wk_v[:, 0:WC])
        wk_copy(1).wait()
        u1 = _dot(x_v[0:R, :], wk_v[:, WC:2 * WC])
        x_copy(0, 1).wait()
        c21 = _dot(x_v[HS:HS + R, :], wk_v[:, 0:HD])
        wk_copy(2).wait()
        wk_copy(3).wait()
        c12 = _dot(x_v[0:R, :], wk_v[:, HD:D])
        ref_forms(wk_v, wks_v, 0, HD, HD, False)
    with _Scope("k1"):
        x_copy(1, 0).wait()
        x_copy(1, 1).wait()
        c22 = _dot(x_v[HS:HS + R, :], wk_v[:, HD:D])
        k_epi(0, (jnp.concatenate([u0, u1], axis=1), c12, c21, c22))
        make_x_forms(1)
        head = _strassen_head(k_prod(1))
    with _Scope("k23_g1"):
        for j in range(2, NP):
            x_copy(j, 0).wait()
            x_copy(j, 1).wait()
        cp_wr.wait()
        cp_gw.wait()
        k_epi(1, _strassen_tail(k_prod(1), head))
        make_x_forms(2)
        k_epi(2, _strassen(k_prod(2)))
        make_x_forms(3)
        k_epi(3, _strassen(k_prod(3)))
        make_x_forms(0)

        z = jnp.sum(jnp.concatenate(zacc, axis=1), axis=0, keepdims=True)
        zc_v[...] = jnp.broadcast_to(z, (BLK, D)).T

        wr = jnp.broadcast_to(wr_v[...].astype(f32).reshape(1, D), (16, D))
        gw = jnp.broadcast_to(gw_v[...].astype(f32).reshape(1, D), (16, D))
        vecs = jnp.where(rid == 0, wr, jnp.where(rid == 1, gw, 0.0)).astype(bf16)
        sc = _dot(vecs, x_v[...], _NT)
        gate_v[...] = jnp.broadcast_to(_sigmoid(sc[1:2, :]), (BLK, S)).T
        r = sc[0:1, :].astype(bf16).astype(f32)
        r_max = jnp.max(r, axis=1, keepdims=True)
        lane = lax.broadcasted_iota(jnp.int32, (1, S), 1)
        idx_v = jnp.min(jnp.where(r == r_max, lane, S), axis=1, keepdims=True)
        idx = jnp.clip(idx_v[0, 0], 0, S - 1)
        base = pl.multiple_of((idx // 16) * 16, 16)
        slab = x_v[pl.ds(base, 16), :].astype(f32)
        x_sel = jnp.sum(jnp.where(rid == idx - base, slab, 0.0), axis=0, keepdims=True)
        xc_v[...] = jnp.broadcast_to(x_sel, (BLK, D)).T

        def g_prod(i):
            return _dot(pks_v[A_FORM[i]], x_form(B_FORM[i], 0, HS))

        m3 = g_prod(2)
        m5 = g_prod(4)
        g_v[0:HD, HD:D] = (m3 + m5).astype(bf16)
        m4 = g_prod(3)
        m1 = g_prod(0)
        t11 = (m1 + m4) - m5
        t22 = m1 + m3

    def q_prod(j):
        return lambda i: _dot(wqs_v[B_FORM[i]], x_form(A_FORM[i], j * R, R), _NT)

    def q_epi(j, c):
        ps = []
        for t, half in zip(c, (0, 1, 0, 1)):
            pq = _phi(t)
            zc = jnp.tile(zc_v[half * HD:(half + 1) * HD, :], (1, R // BLK))
            den = jnp.sum((pq * zc).reshape(H // 2, DH, R), axis=1, keepdims=True) + 1e-6
            ps.append((pq.reshape(H // 2, DH, R) * (1.0 / den)).reshape(HD, R))
        fs = _forms(*ps)
        for f in range(7):
            ps_v[f, :, j * R:(j + 1) * R] = fs[f].astype(bf16)

    with _Scope("g2"):
        cp_wg.wait()
        cp_wu.wait()
        cp_wq.wait()
        m2 = g_prod(1)
        g_v[HD:D, 0:HD] = (m2 + m4).astype(bf16)
        g_v[0:HD, 0:HD] = (t11 + g_prod(6)).astype(bf16)
        g_v[HD:D, HD:D] = ((t22 - m2) + g_prod(5)).astype(bf16)
        make_wq_forms()
        head = _strassen_head(q_prod(0))

        gg, uu = _matvec_chains((wg_v, wu_v), xc_v, D, F, live)

    with _Scope("mid_q01"):
        cp_wv.wait()
        cp_wo.wait()
        hh = gg * _sigmoid(gg) * uu
        hc_v[...] = jnp.broadcast_to(hh, (BLK, F)).T
        c = _strassen_tail(q_prod(0), head)
        ri = lax.broadcasted_iota(jnp.int32, (BLK, BLK), 0) // DH
        ci = lax.broadcasted_iota(jnp.int32, (BLK, BLK), 1) // DH
        diag = ri == ci
        kvs = []
        for j in range(NB):
            sl = slice(j * BLK, (j + 1) * BLK)
            kv = _dot(g_v[sl, :], wv_v[:, sl])
            kvs.append(jnp.where(diag, kv, 0.0).astype(bf16))
        q_epi(0, c)
        for j in range(NB // 2):
            j2 = j + NB // 2
            mu = _dot(kvs[j], wo_v[j * BLK:(j + 1) * BLK, :])
            ml = _dot(kvs[j2], wo_v[j2 * BLK:(j2 + 1) * BLK, :])
            fs = _forms(mu[:, :HD], mu[:, HD:], ml[:, :HD], ml[:, HD:])
            for f in range(7):
                ms_v[f, j * BLK:(j + 1) * BLK, :] = fs[f].astype(bf16)
        head = _strassen_head(q_prod(1))
    with _Scope("rest"):
        cp_wd.wait()
        q_epi(1, _strassen_tail(q_prod(1), head))
        q_epi(2, _strassen(q_prod(2)))
        q_epi(3, _strassen(q_prod(3)))

        (yy,) = _matvec_chains((wd_v,), hc_v, F, D, live)
        y = yy * _sigmoid(r_max)

        def mix(i, half, col, a):
            r0, n = A_PIECES[i]
            r0 = r0 + half * HS
            cs = slice(col * HD, (col + 1) * HD)
            g = jnp.tile(gate_v[r0:r0 + n, :], (1, HD // BLK))
            rows = lax.broadcasted_iota(jnp.int32, (n, HD), 0) + r0
            b = x_v[r0:r0 + n, cs].astype(f32) + jnp.where(rows == idx, y[:, cs], 0.0)
            out_v[r0:r0 + n, cs] = (g * a + (1.0 - g) * b).astype(bf16)
            out_copy(i, half, col).start()

        for i, (r0, n) in enumerate(A_PIECES):
            c11, c12, c21, c22 = _strassen(
                lambda m: _dot(ps_v[A_FORM[m], :, r0:r0 + n], ms_v[B_FORM[m]], _TN))
            mix(i, 0, 1, c12)
            mix(i, 1, 0, c21)
            mix(i, 0, 0, c11)
            mix(i, 1, 1, c22)
        for i in range(len(A_PIECES)):
            for half in range(2):
                for col in range(2):
                    out_copy(i, half, col).wait()


@jax.jit
def pallas_gated_mix__linear_attn_block__moe_arch_mod__prompt_kernel(
    A_x: jax.Array,
    A_wqkv: jax.Array,
    A_wo: jax.Array,
    B_x: jax.Array,
    B_w_r: jax.Array,
    B_w_gate: jax.Array,
    B_w_up: jax.Array,
    B_w_down: jax.Array,
    gate_w: jax.Array,
):
    del B_x
    any_spec = pl.BlockSpec(memory_space=pl.ANY)
    scratch = [
        pltpu.VMEM((S, D), bf16),
        pltpu.VMEM((D, D), bf16),
        pltpu.VMEM((D, D), bf16),
        pltpu.VMEM((D, D), bf16),
        pltpu.VMEM((D, D), bf16),
        pltpu.VMEM((D, F), bf16),
        pltpu.VMEM((D, F), bf16),
        pltpu.VMEM((F, D), bf16),
        pltpu.VMEM((D,), bf16),
        pltpu.VMEM((D,), bf16),
        pltpu.VMEM((5, HS, HD), bf16),
        pltpu.VMEM((5, HD, HD), bf16),
        pltpu.VMEM((7, HD, HD), bf16),
        pltpu.VMEM((7, HD, HS), bf16),
        pltpu.VMEM((D, D), bf16),
        pltpu.VMEM((7, HD, HD), bf16),
        pltpu.VMEM((7, HD, HS), bf16),
        pltpu.VMEM((S, D), bf16),
        pltpu.VMEM((S, BLK), f32),
        pltpu.VMEM((D, BLK), f32),
        pltpu.VMEM((D, BLK), f32),
        pltpu.VMEM((F, BLK), f32),
        pltpu.SemaphoreType.DMA((D // WC + 2 * NP,)),
        pltpu.SemaphoreType.DMA((8,)),
        pltpu.SemaphoreType.DMA((4 * len(A_PIECES),)),
    ]
    return pl.pallas_call(
        _kernel,
        out_shape=jax.ShapeDtypeStruct((1, S, D), bf16),
        in_specs=[any_spec] * 8,
        out_specs=any_spec,
        scratch_shapes=scratch,
        compiler_params=pltpu.CompilerParams(vmem_limit_bytes=120 * 1024 * 1024),
    )(A_x, A_wqkv, A_wo, B_w_r, B_w_gate, B_w_up, B_w_down, gate_w)
```

```python
import functools
import os
import jax
import jax.numpy as jnp
from jax import lax
import jax.experimental.pallas as pl
import jax.experimental.pallas.tpu as pltpu

S = 2048
D = 1024
F = 3584
H = 32
DH = D // H
HS = S // 2
HD = D // 2
R = 256
NP = HS // R
BLK = 128
NB = D // BLK
WC = 256
NK = D // WC

SCOPES = os.environ.get("K_SCOPES", "0") == "1"
OPT = dict(kv.split("=") for kv in os.environ.get("K_OPT", "").split(",") if kv)

_NN = (((1,), (0,)), ((), ()))
_NT = (((1,), (1,)), ((), ()))
_TN = (((0,), (0,)), ((), ()))
f32 = jnp.float32
bf16 = jnp.bfloat16
u32 = jnp.uint32
OC = 256


A_FORM = (0, 1, 5, 6, 2, 3, 4)
B_FORM = (0, 5, 4, 3, 6, 2, 1)


def _forms(b11, b12, b21, b22):
    return (b11 + b22, b21 + b22, b11 + b12, b21 - b11, b12 - b22, b11, b22)


def _strassen_head(prod, post):
    m3 = prod(2)
    m4 = prod(3)
    m5 = prod(4)
    p12 = post(m3 + m5, 1, 0)
    m2 = prod(1)
    p21 = post(m2 + m4, 0, 1)
    m1 = prod(0)
    return p12, p21, (m1 + m4) - m5, (m1 - m2) + m3


def _strassen_tail(prod, post, head):
    p12, p21, t11, t22 = head
    p11 = post(t11 + prod(6), 0, 0)
    p22 = post(t22 + prod(5), 1, 1)
    return p11, p12, p21, p22


def _strassen_head2(prod):
    m3 = prod(2)
    m4 = prod(3)
    m1 = prod(0)
    t11 = (m1 + m4) + prod(6)
    t22 = (m1 + m3) + prod(5)
    return m3, m4, t11, t22


def _strassen_tail2(prod, post, head):
    m3, m4, t11, t22 = head
    m5 = prod(4)
    p12 = post(m3 + m5, 1, 0)
    p11 = post(t11 - m5, 0, 0)
    m2 = prod(1)
    p21 = post(m2 + m4, 0, 1)
    p22 = post(t22 - m2, 1, 1)
    return p11, p12, p21, p22


def _strassen(prod, post):
    return _strassen_tail(prod, post, _strassen_head(prod, post))


def _pk(a):
    return pltpu.bitcast(a.astype(bf16), u32)


def _unpk(a):
    return pltpu.bitcast(a, bf16)


def _link(live, prev):
    return jnp.where(live, 0.0, prev)


def _chained_forms(blocks, live, prev, pad):
    halves = []
    for h in range(2):
        b11, b12, b21, b22 = (b[8 * h:8 * (h + 1)] for b in blocks)
        b11 = b11 + _link(live, prev)
        s1112 = b11 + b12
        s2122 = b21 + b22
        prev = s1112 + s2122
        for _ in range(pad):
            prev = prev + s2122
        halves.append((b11 + b22, s2122, s1112, b21 - b11, b12 - b22, b11, b22))
    forms = [_pk(jnp.concatenate([halves[0][f], halves[1][f]], axis=0)) for f in range(7)]
    return forms, prev


def _recip(d):
    if OPT.get("nr", "2") == "e":
        r = pl.reciprocal(d, approx=True)
        return r * (2.0 - d * r)
    if OPT.get("nr", "2") == "e0":
        return pl.reciprocal(d, approx=True)
    r = pltpu.bitcast(jnp.int32(0x7EF311C3) - pltpu.bitcast(d, jnp.int32), f32)
    if OPT.get("nr", "2") == "2":
        r = r * (2.00130856 - d * r)
        return r * (2.00000084 - d * r)
    for _ in range(3):
        r = r * (2.0 - d * r)
    return r


def _tree_sum(vals):
    while len(vals) > 1:
        vals = [sum(vals[i + 1:i + 2], vals[i]) for i in range(0, len(vals), 2)]
    return vals[0]


def _pad_chain(live, prev, n):
    for _ in range(n):
        prev = _link(live, prev)
    return prev


def _dot(a, b, dims=_NN):
    return lax.dot_general(a, b, dims, preferred_element_type=f32)


def _phi(t):
    return jnp.where(t > 0, t + 1.0, jnp.exp(t)) + 1e-6


def _sigmoid(t):
    return 1.0 / (1.0 + jnp.exp(-t))


class _Scope:
    def __init__(self, name):
        self.c = jax.named_scope(name) if SCOPES else None
    def __enter__(self):
        if self.c is not None:
            self.c.__enter__()
    def __exit__(self, *a):
        if self.c is not None:
            self.c.__exit__(*a)


def _matvec_chain(w_refs, col_ref, n_rows, n_cols, live, width, prev):
    rep = width // BLK
    outs = [[] for _ in w_refs]
    for c0 in range(0, n_cols, width):
        for w_ref, out in zip(w_refs, outs):
            def step(i, acc, w_ref=w_ref):
                r0 = pl.multiple_of(i * 8, 8)
                col = col_ref[pl.ds(r0, 8), :]
                w = w_ref[pl.ds(r0, 8), c0:c0 + width].astype(f32)
                return acc + w * jnp.concatenate([col] * rep, axis=1)
            link = _link(live, prev)
            acc = lax.fori_loop(0, n_rows // 8, step, jnp.concatenate([link] * rep, axis=1),
                                unroll=True)
            out.append(acc)
            prev = acc[:, 0:BLK]
            for h in range(1, rep):
                prev = prev + acc[:, h * BLK:(h + 1) * BLK]
    return [jnp.concatenate(o, axis=1) for o in outs], prev


SCRATCH = dict(
    x_v=((S, D), bf16), wq_v=((D, D), bf16), wk_v=((D, D), bf16), wv_v=((D, D), bf16),
    wo_v=((D, D), bf16), wg_v=((D, F), bf16), wu_v=((D, F), bf16), wd_v=((F, D), bf16),
    wr_v=((D,), bf16), gw_v=((D,), bf16),
    xs_v=((5, HS // 2, HD), u32),
    wks_v=((5, HD // 2, HD), u32),
    wqs_v=((7, HD // 2, HD), u32),
    pks_v=((7, HD // 2, HS), u32),
    g_v=((D // 2, D), u32),
    ms_v=((7, HD // 2, HD), u32),
    ps_v=((7, HS // 2, HD), u32),
    out_v=((S, D), bf16),
    gate_v=((S, BLK), f32),
    zc_v=((D, BLK), f32),
    xc_v=((D, BLK), f32),
    hc_v=((F, BLK), f32),
    ck_v=((4, R, HD), f32),
    cq_v=((4, HD, R), f32),
    cg_v=((3, HD, HD), f32),
    wb_v=((2, 8, D), f32),
    c0_v=((4, R, HD), f32),
    gu_v=((2, 8, F), f32),
    sel_v=((2, 8, BLK), f32),
)


OUT_ORDER = tuple(tuple(half * HS + r0 for r0 in range(0, HS, R) for half in ((1, 0), (0, 1))[col])
                  for col in range(2))


def _blocks(v, start_out, state):
    x_v, wk_v, wq_v = v["x_v"], v["wk_v"], v["wq_v"]
    xs_v, wks_v, wqs_v, pks_v, ms_v, ps_v = (v[k] for k in (
        "xs_v", "wks_v", "wqs_v", "pks_v", "ms_v", "ps_v"))
    ck_v, cq_v, cg_v, c0_v, gu_v, sel_v = (v[k] for k in (
        "ck_v", "cq_v", "cg_v", "c0_v", "gu_v", "sel_v"))
    g_v, gate_v, zc_v, xc_v, hc_v, out_v = (v[k] for k in (
        "g_v", "gate_v", "zc_v", "xc_v", "hc_v", "out_v"))
    zero = jnp.zeros((8, BLK), f32)

    def get_live():
        words = pltpu.bitcast(x_v[0:16, 0:BLK], jnp.int32)
        return lax.shift_right_arithmetic(words, 31) >= -1

    def x_form(f, r0, n):
        if f == 5:
            return x_v[r0:r0 + n, 0:HD]
        if f == 6:
            return x_v[HS + r0:HS + r0 + n, HD:D]
        return _unpk(xs_v[f, r0 // 2:(r0 + n) // 2, :])

    def sel_idx():
        if "idx" not in state:
            state["idx"] = sel_v[1, 0:1, 0:1].astype(jnp.int32)[0, 0]
        return state["idx"]

    def wk_form(f):
        if f == 5:
            return wk_v[0:HD, 0:HD]
        if f == 6:
            return wk_v[HD:D, HD:D]
        return _unpk(wks_v[f])

    def free_forms(src, dst, r0, n, half_rows, f):
        for r in range(r0, r0 + n, 16):
            for c in range(0, HD, 2 * BLK):
                blocks = [jnp.concatenate([src[rr:rr + 8, cc:cc + 2 * BLK].astype(f32),
                                           src[rr + 8:rr + 16, cc:cc + 2 * BLK].astype(f32)], axis=0)
                          for rr in (r, half_rows + r) for cc in (c, HD + c)]
                dst[f, r // 2:r // 2 + 8, c:c + 2 * BLK] = _pk(_forms(*blocks)[f])

    def make_wq_forms(live, pad):
        prev = zero
        for r in range(0, HD, BLK):
            for c in range(0, HD, 2 * BLK):
                tiles = [wq_v[rr:rr + 2 * BLK, cc:cc + BLK].T
                         for rr, cc in ((c, r), (c, HD + r), (HD + c, r), (HD + c, HD + r))]
                for s0 in range(0, BLK, 16):
                    for c1 in range(0, 2 * BLK, BLK):
                        blocks = [t[s0:s0 + 16, c1:c1 + BLK].astype(f32) for t in tiles]
                        fs, prev = _chained_forms(blocks, live, prev, pad)
                        for f in range(7):
                            wqs_v[f, (r + s0) // 2:(r + s0) // 2 + 8, c + c1:c + c1 + BLK] = fs[f]
        return prev

    def anchored(prod, i, ref, f, live, prev):
        def wrapped(m):
            if m == i:
                link = jnp.concatenate([_link(live, prev)] * 2, axis=0)
                ref[f, 0:8, 0:BLK] = _pk(_unpk(ref[f, 0:8, 0:BLK]).astype(f32) + link)
            return prod(m)
        return wrapped

    def last_rows(t):
        out = []
        for r in range(BLK, t.shape[0] + 1, BLK):
            last = t[r - 16:r, :].astype(f32)[8:16]
            out += [last[:, c:c + BLK] for c in range(0, t.shape[1], BLK)]
        return _tree_sum(out)

    def k_post(c, col, half):
        return _phi(c)

    done = []

    def k_epi(j, p, z):
        p11, p12, p21, p22 = p
        zs = jnp.concatenate([jnp.sum((p11 + p21).reshape(R // 8, 8, HD), axis=0),
                              jnp.sum((p12 + p22).reshape(R // 8, 8, HD), axis=0)], axis=1)
        fs = _forms(p11, p21, p12, p22)
        for f in (5, 2, 6, 0, 1, 4, 3):
            t = fs[f].astype(bf16).T
            pks_v[f, :, j * R:(j + 1) * R] = _pk(t)
            done.append(last_rows(t))
        return zs if z is None else z + zs

    def k_prod(j):
        return lambda i: _dot(x_form(A_FORM[i], j * R, R), wk_form(B_FORM[i]))

    def g_prod(i, k0=0, k1=HS):
        return _dot(_unpk(pks_v[A_FORM[i], :, k0:k1]), x_form(B_FORM[i], k0, k1 - k0))

    def q_prod(j):
        return lambda i: _dot(_unpk(wqs_v[B_FORM[i]]), x_form(A_FORM[i], j * R, R), _NT)

    def q_post(c, col, half):
        pq = _phi(c)
        zc = jnp.tile(zc_v[col * HD:(col + 1) * HD, :], (1, R // BLK))
        w = (pq * zc).reshape(H // 2, DH // 8, 8, R)
        if OPT.get("eps", "1") == "1":
            eps = jnp.where(lax.broadcasted_iota(jnp.int32, (8, R), 0) == 0, 1e-6, 0.0)
            part = ((w[:, 0] + eps) + w[:, 1]) + w[:, 2] + w[:, 3]
            if OPT.get("r4", "0") == "1":
                p2 = part.reshape(H // 2 * 8, R)
                p2 = jnp.concatenate([pltpu.roll(p2[8 * h:8 * h + 8], 4, 0) + p2[8 * h:8 * h + 8] for h in range(H // 2)], axis=0)
                def r3(a):
                    return (a + pltpu.roll(a, 1, 0)) + (pltpu.roll(a, 2, 0) + pltpu.roll(a, 3, 0))
                inv = _recip(jnp.concatenate([r3(p2[8 * h:8 * h + 8]) for h in range(H // 2)], axis=0))
                return (pq.reshape(H // 2, DH // 8, 8, R) * inv.reshape(H // 2, 1, 8, R)).reshape(HD, R)
            den = jnp.sum(part, axis=1, keepdims=True)
        else:
            den = jnp.sum(w[:, 0] + w[:, 1] + w[:, 2] + w[:, 3], axis=1, keepdims=True) + 1e-6
        return (pq.reshape(H // 2, DH, R) * _recip(den)).reshape(HD, R)

    def q_epi(j, p):
        fs = _forms(*p)
        ends = []
        for f in range(7):
            t = fs[f].astype(bf16).T
            ps_v[f, j * R // 2:(j + 1) * R // 2, :] = _pk(t)
            ends.append(last_rows(t))
        return _tree_sum(ends)

    def b0():
        c0_v[0, :, 0:WC] = _dot(x_v[0:R, :], wk_v[:, 0:WC])

    def b1():
        c0_v[0, :, WC:HD] = _dot(x_v[0:R, :], wk_v[:, WC:HD])

    def b2():
        c0_v[2] = _dot(x_v[HS:HS + R, :], wk_v[:, 0:HD])

    def b3():
        c0_v[1] = _dot(x_v[0:R, :], wk_v[:, HD:D])

    def b4():
        c0_v[3] = _dot(x_v[HS:HS + R, :], wk_v[:, HD:D])
        for f in (4, 3, 0, 1, 2):
            free_forms(wk_v, wks_v, 0, HD, HD, f)
        sep_forms(1, (0, 4, 3))
        head = _strassen_head2(k_prod(1))
        for i in range(4):
            ck_v[i] = head[i]

    def sep_forms(j, which):
        for f in which:
            free_forms(x_v, xs_v, j * R, R, HS, f)

    def router(live, prev):
        wr_ref, gw_ref = v["wb_v"].at[0], v["wb_v"].at[1]
        v["wb_v"][0] = jnp.broadcast_to(v["wr_v"][...].astype(f32).reshape(1, D), (8, D))
        v["wb_v"][1] = jnp.broadcast_to(v["gw_v"][...].astype(f32).reshape(1, D), (8, D))
        serial = OPT.get("rs", "0") == "1"
        rows, ends = [], []
        for t in range(S // BLK):
            accs = [[], []]
            for r in range(t * BLK, (t + 1) * BLK, 8):
                ar = ag = _link(live, prev)
                for c in range(0, D, 2 * BLK):
                    xx = x_v[r:r + 8, c:c + 2 * BLK].astype(f32)
                    for h in range(2):
                        cs = slice(c + h * BLK, c + (h + 1) * BLK)
                        xh = xx[:, h * BLK:(h + 1) * BLK]
                        ar = ar + xh * wr_ref[:, cs]
                if serial:
                    ag = _link(live, ar)
                for c in range(0, D, 2 * BLK):
                    xx = x_v[r:r + 8, c:c + 2 * BLK].astype(f32)
                    for h in range(2):
                        cs = slice(c + h * BLK, c + (h + 1) * BLK)
                        xh = xx[:, h * BLK:(h + 1) * BLK]
                        ag = ag + xh * gw_ref[:, cs]
                prev = ag if serial else ar + ag
                accs[0].append(ar)
                accs[1].append(ag)
            sums = [jnp.sum(jnp.concatenate(a, axis=0).T, axis=0, keepdims=True) for a in accs]
            rows.append(sums[0])
            gate = jnp.broadcast_to(_sigmoid(sums[1]), (BLK, BLK)).T
            gate_v[t * BLK:(t + 1) * BLK, :] = gate
            ends.append(gate[BLK - 8:])
        r = jnp.concatenate(rows, axis=1).astype(bf16).astype(f32)
        r_max = jnp.max(r, axis=1, keepdims=True)
        lane = lax.broadcasted_iota(jnp.int32, (1, S), 1)
        idx_v = jnp.min(jnp.where(r == r_max, lane, S), axis=1, keepdims=True)
        idx_v = jnp.clip(idx_v, 0, S - 1)
        sel_v[0] = jnp.broadcast_to(_sigmoid(r_max), (8, BLK))
        sel_v[1] = jnp.broadcast_to(idx_v.astype(f32), (8, BLK))
        idx = idx_v[0, 0]
        state["idx"] = idx
        base = pl.multiple_of((idx // 16) * 16, 16)
        slab = x_v[pl.ds(base, 16), :].astype(f32)
        rid = lax.broadcasted_iota(jnp.int32, (16, D), 0)
        x_sel = jnp.sum(jnp.where(rid == idx - base, slab, 0.0), axis=0, keepdims=True)
        xc = jnp.broadcast_to(x_sel, (BLK, D)).T
        xc_v[...] = xc
        return last_slabs(xc) + _tree_sum(ends)

    def last_slabs(a):
        n = a.shape[0] // BLK
        return jnp.sum(a.reshape(n, BLK // 8, 8, BLK)[:, BLK // 8 - 1], axis=0)

    def b5():
        live = get_live()
        sep_forms(1, (2, 1))
        z = k_epi(1, _strassen_tail2(k_prod(1), k_post, [ck_v[i] for i in range(4)]), None)
        z = k_epi(0, [_phi(c0_v[i]) for i in range(4)], z)
        sep_forms(2, (2, 1, 0, 4, 3))
        z = k_epi(2, _strassen(k_prod(2), k_post), z)
        sep_forms(3, (2, 1, 0, 4, 3))
        z = k_epi(3, _strassen(k_prod(3), k_post), z)
        z = jnp.sum(z, axis=0, keepdims=True)
        zc = jnp.broadcast_to(z, (BLK, D)).T
        zc_v[...] = zc
        sep_forms(0, (4, 3, 0))
        end = router(live, _tree_sum(done) + last_slabs(zc))

        m3 = g_prod(2, R, HS - R) + g_prod(2, 0, R) + g_prod(2, HS - R, HS)
        m5 = g_prod(4)
        g_v[0:HD // 2, HD:D] = _pk(m3 + m5)
        m4 = g_prod(3)
        m1 = g_prod(0)
        link = jnp.concatenate([_link(live, end)] * (HD // BLK), axis=1)
        m1 = jnp.concatenate([m1[:HD - 8], m1[HD - 8:] + link], axis=0)
        cg_v[0] = m4
        cg_v[1] = (m1 + m4) - m5
        cg_v[2] = m1 + m3

    def b6():
        live = get_live()
        sep_forms(0, (1, 2))
        m2 = g_prod(1)
        g_v[HD // 2:D // 2, 0:HD] = _pk(m2 + cg_v[0])
        g_v[0:HD // 2, 0:HD] = _pk(cg_v[1] + g_prod(6))
        g_v[HD // 2:D // 2, HD:D] = _pk((cg_v[2] - m2) + g_prod(5))
        end = make_wq_forms(live, int(OPT.get("wq", 4)))
        (gg, uu), end = _matvec_chain((v["wg_v"], v["wu_v"]), xc_v, D, F, live,
                                      int(OPT.get("gu", 256)), end)
        gu_v[0] = gg
        gu_v[1] = uu
        head = _strassen_head(anchored(q_prod(0), 1, wqs_v, B_FORM[1], live, end), q_post)
        for i in range(4):
            cq_v[i] = head[i]

    def a_prod(j):
        return lambda m: _dot(_unpk(ps_v[A_FORM[m], j * R // 2:(j + 1) * R // 2, :]),
                              _unpk(ms_v[B_FORM[m]]))

    def a_post(j):
        def post(a, col, half):
            rr = j * R + half * HS
            cs = slice(col * HD, (col + 1) * HD)
            g = jnp.tile(gate_v[rr:rr + R, :], (1, HD // BLK))
            b = x_v[rr:rr + R, cs].astype(f32)
            out_v[rr:rr + R, cs] = (g * a + (1.0 - g) * b).astype(bf16)
            k = OUT_ORDER[col].index(rr)
            if k:
                for c in range(col * HD, (col + 1) * HD, OC):
                    start_out(c, k)
        return post

    def b7():
        live = get_live()
        sel_idx()
        gg = jnp.sum(gu_v[0], axis=0, keepdims=True)
        uu = jnp.sum(gu_v[1], axis=0, keepdims=True)
        hh = gg * _sigmoid(gg) * uu
        hc = jnp.broadcast_to(hh, (BLK, F)).T
        hc_v[...] = hc
        p = _strassen_tail(q_prod(0), q_post, [cq_v[i] for i in range(4)])
        ri = lax.broadcasted_iota(jnp.int32, (BLK, BLK), 0) // DH
        ci = lax.broadcasted_iota(jnp.int32, (BLK, BLK), 1) // DH
        diag = ri == ci
        kvs = []
        for j in range(NB):
            sl = slice(j * BLK, (j + 1) * BLK)
            kv = _dot(_unpk(g_v[j * BLK // 2:(j + 1) * BLK // 2, :]), v["wv_v"][:, sl])
            kvs.append(jnp.where(diag, kv, 0.0).astype(bf16))
        q_epi(0, p)
        for j in range(NB // 2):
            j2 = j + NB // 2
            mu = _dot(kvs[j], v["wo_v"][j * BLK:(j + 1) * BLK, :])
            ml = _dot(kvs[j2], v["wo_v"][j2 * BLK:(j2 + 1) * BLK, :])
            fs = _forms(mu[:, :HD], mu[:, HD:], ml[:, :HD], ml[:, HD:])
            for f in range(7):
                ms_v[f, j * BLK // 2:(j + 1) * BLK // 2, :] = _pk(fs[f])
        ends = [q_epi(1, _strassen(anchored(q_prod(1), 2, wqs_v, B_FORM[2], live, last_slabs(hc)),
                                   q_post)),
                q_epi(2, _strassen(q_prod(2), q_post)),
                q_epi(3, _strassen(q_prod(3), q_post))]
        prod = a_prod(0)
        if OPT.get("pa", "1") == "1":
            prod = anchored(prod, 0, ms_v, B_FORM[0], live, _tree_sum(ends))
        head = _strassen_head(prod, a_post(0))
        ck_v[0] = head[2]
        ck_v[1] = head[3]

    def b8():
        live = get_live()
        idx = sel_idx()
        (yy,), end = _matvec_chain((v["wd_v"],), hc_v, F, D, live, int(OPT.get("dn", 128)), zero)
        y = jnp.sum(yy, axis=0, keepdims=True) * sel_v[0, 0:1, 0:1]

        _strassen_tail(a_prod(0), a_post(0), (None, None, ck_v[0], ck_v[1]))
        for j in range(1, NP):
            prod = a_prod(j)
            if j == int(OPT.get("dnp", 3)):
                prod = anchored(prod, 2, ms_v, B_FORM[2], live, end)
            _strassen(prod, a_post(j))

        base = pl.multiple_of((idx // 16) * 16, 16)
        g = jnp.tile(gate_v[pl.ds(base, 16), :], (1, NB))
        rid = lax.broadcasted_iota(jnp.int32, (16, D), 0)
        upd = jnp.where(rid == idx - base, (1.0 - g) * y, 0.0)
        out_v[pl.ds(base, 16), :] = (out_v[pl.ds(base, 16), :].astype(f32) + upd).astype(bf16)
        for c in range(0, D, OC):
            start_out(c, 0)

    return [b0, b1, b2, b3, b4, b5, b6, b7, b8]


def _out_copy(src, dst, sems, idx, c, k):
    order = OUT_ORDER[c // HD]
    blk = (idx // R) * R
    if k == 0:
        r0 = blk
    else:
        seen = functools.reduce(jnp.logical_or, [blk == r for r in order[:k]])
        r0 = jnp.where(seen, order[k], order[k - 1])
    r0 = pl.multiple_of(r0, R)
    return pltpu.make_async_copy(src.at[pl.ds(r0, R), pl.ds(c, OC)], dst.at[pl.ds(r0, R), pl.ds(c, OC)],
                                 sems.at[c // OC, k])


def _kernel(x_hbm, wqkv_hbm, wo_hbm, wr_hbm, wg_hbm, wu_hbm, wd_hbm, gw_hbm,
            out_hbm, *scratch):
    v = dict(zip(SCRATCH, scratch))
    sem_hi, sem_lo, sem_o = scratch[len(SCRATCH):]

    def x_copy(j, half):
        r0 = half * HS + j * R
        return pltpu.make_async_copy(x_hbm.at[0, pl.ds(r0, R), :],
                                     v["x_v"].at[pl.ds(r0, R), :],
                                     sem_hi.at[NK + 2 * j + half])

    def wk_copy(c):
        return pltpu.make_async_copy(wqkv_hbm.at[:, pl.ds(D + c * WC, WC)],
                                     v["wk_v"].at[:, pl.ds(c * WC, WC)], sem_hi.at[c])

    cp_wq = pltpu.make_async_copy(wqkv_hbm.at[:, pl.ds(0, D)], v["wq_v"], sem_lo.at[0])
    cp_wv = pltpu.make_async_copy(wqkv_hbm.at[:, pl.ds(2 * D, D)], v["wv_v"], sem_lo.at[1])
    cp_wo = pltpu.make_async_copy(wo_hbm, v["wo_v"], sem_lo.at[2])
    cp_wg = pltpu.make_async_copy(wg_hbm, v["wg_v"], sem_lo.at[3])
    cp_wu = pltpu.make_async_copy(wu_hbm, v["wu_v"], sem_lo.at[4])
    cp_wd = pltpu.make_async_copy(wd_hbm, v["wd_v"], sem_lo.at[5])
    cp_wr = pltpu.make_async_copy(wr_hbm, v["wr_v"], sem_lo.at[6])
    cp_gw = pltpu.make_async_copy(gw_hbm, v["gw_v"], sem_lo.at[7])

    state = {}

    def out_copy(c, k):
        return _out_copy(v["out_v"], out_hbm.at[0], sem_o, state["idx"], c, k)

    x_copy(0, 0).start()
    wk_copy(0).start()
    wk_copy(1).start()
    x_copy(0, 1).start()
    wk_copy(2).start()
    wk_copy(3).start()
    for j in range(1, NP):
        x_copy(j, 0).start()
        x_copy(j, 1).start()
    for cp in (cp_wr, cp_gw, cp_wg, cp_wu, cp_wq, cp_wv, cp_wo, cp_wd):
        cp.start(priority=1)

    waits = [
        [x_copy(0, 0), wk_copy(0)],
        [wk_copy(1)],
        [x_copy(0, 1)],
        [wk_copy(2), wk_copy(3)],
        [x_copy(1, 0), x_copy(1, 1)],
        [x_copy(j, h) for j in range(2, NP) for h in range(2)] + [cp_wr, cp_gw],
        [cp_wg, cp_wu, cp_wq],
        [cp_wv, cp_wo],
        [cp_wd],
    ]
    blocks = _blocks(v, lambda c, k: out_copy(c, k).start(), state)
    for n, (ws, blk) in enumerate(zip(waits, blocks)):
        with _Scope(f"w{n}"):
            for cp in ws:
                cp.wait()
        with _Scope(f"b{n}"):
            blk()
    with _Scope("w9"):
        for k in list(range(1, S // R)) + [0]:
            for c in range(0, D, OC):
                out_copy(c, k).wait()


@jax.jit
def pallas_gated_mix__linear_attn_block__moe_arch_mod__prompt_kernel(
    A_x: jax.Array,
    A_wqkv: jax.Array,
    A_wo: jax.Array,
    B_x: jax.Array,
    B_w_r: jax.Array,
    B_w_gate: jax.Array,
    B_w_up: jax.Array,
    B_w_down: jax.Array,
    gate_w: jax.Array,
):
    del B_x
    any_spec = pl.BlockSpec(memory_space=pl.ANY)
    scratch = [pltpu.VMEM(*s) for s in SCRATCH.values()] + [
        pltpu.SemaphoreType.DMA((NK + 2 * NP,)),
        pltpu.SemaphoreType.DMA((8,)),
        pltpu.SemaphoreType.DMA((D // OC, S // R)),
    ]
    return pl.pallas_call(
        _kernel,
        out_shape=jax.ShapeDtypeStruct((1, S, D), bf16),
        in_specs=[any_spec] * 8,
        out_specs=any_spec,
        scratch_shapes=scratch,
        compiler_params=pltpu.CompilerParams(vmem_limit_bytes=120 * 1024 * 1024),
    )(A_x, A_wqkv, A_wo, B_w_r, B_w_gate, B_w_up, B_w_down, gate_w)
```

```python
import functools
import jax
import jax.numpy as jnp
from jax import lax
import jax.experimental.pallas as pl
import jax.experimental.pallas.tpu as pltpu

S = 2048
D = 1024
F = 3584
H = 32
DH = D // H
HS = S // 2
HD = D // 2
R = 256
NP = HS // R
BLK = 128
NB = D // BLK
K_CHUNKS = ((0, 128), (128, 128), (256, 256), (512, 256), (768, 256))
NK = len(K_CHUNKS)

_NN = (((1,), (0,)), ((), ()))
_NT = (((1,), (1,)), ((), ()))
_TN = (((0,), (0,)), ((), ()))
f32 = jnp.float32
bf16 = jnp.bfloat16
u32 = jnp.uint32


A_FORM = (0, 1, 5, 6, 2, 3, 4)
B_FORM = (0, 5, 4, 3, 6, 2, 1)


def _forms(b11, b12, b21, b22):
    return (b11 + b22, b21 + b22, b11 + b12, b21 - b11, b12 - b22, b11, b22)


def _strassen_head(prod, post):
    m3 = prod(2)
    m4 = prod(3)
    m5 = prod(4)
    p12 = post(m3 + m5, 1, 0)
    m2 = prod(1)
    p21 = post(m2 + m4, 0, 1)
    m1 = prod(0)
    return p12, p21, (m1 + m4) - m5, (m1 - m2) + m3


def _strassen_tail(prod, post, head):
    p12, p21, t11, t22 = head
    p11 = post(t11 + prod(6), 0, 0)
    p22 = post(t22 + prod(5), 1, 1)
    return p11, p12, p21, p22


def _strassen_head2(prod):
    m5 = prod(4)
    m2 = prod(1)
    m1 = prod(0)
    t11 = (m1 - m5) + prod(6)
    t22 = (m1 - m2) + prod(5)
    return m5, m2, t11, t22


def _strassen_tail2(prod, post, head):
    m5, m2, t11, t22 = head
    m3 = prod(2)
    p12 = post(m3 + m5, 1, 0)
    p22 = post(t22 + m3, 1, 1)
    m4 = prod(3)
    p21 = post(m2 + m4, 0, 1)
    p11 = post(t11 + m4, 0, 0)
    return p11, p12, p21, p22


def _strassen(prod, post):
    return _strassen_tail(prod, post, _strassen_head(prod, post))


def _pk(a):
    return pltpu.bitcast(a.astype(bf16), u32)


def _unpk(a):
    return pltpu.bitcast(a, bf16)


class _Packed:
    def __init__(self, ref, rows):
        self.ref, self.rows = ref, rows

    def _idx(self, f, r0, n, c0, c1):
        n = self.rows - r0 if n is None else n
        a = (f * self.rows + r0) // 2
        return slice(a, a + n // 2), slice(c0, c1)

    def get(self, f, r0=0, n=None, c0=None, c1=None):
        return _unpk(self.ref[self._idx(f, r0, n, c0, c1)])

    def put(self, val, f, r0=0, c0=0):
        self.ref[self._idx(f, r0, val.shape[0], c0, c0 + val.shape[1])] = _pk(val)


def _link(live, prev):
    return jnp.where(live, 0.0, prev)


def _chained_forms(blocks, live, prev, pad):
    b11, b12, b21, b22 = blocks
    b11 = b11 + _link(live, prev)
    s1112 = b11 + b12
    s2122 = b21 + b22
    prev = s1112 + s2122
    for _ in range(pad):
        prev = prev + s2122
    return (b11 + b22, s2122, s1112, b21 - b11, b12 - b22, b11, b22), prev


def _recip(d):
    r = pltpu.bitcast(jnp.int32(0x7EF311C3) - pltpu.bitcast(d, jnp.int32), f32)
    r = r * (2.00130856 - d * r)
    return r * (2.00000084 - d * r)


def _tree_sum(vals):
    while len(vals) > 1:
        vals = [sum(vals[i + 1:i + 2], vals[i]) for i in range(0, len(vals), 2)]
    return vals[0]


def _dot(a, b, dims=_NN):
    return lax.dot_general(a, b, dims, preferred_element_type=f32)


def _phi(t):
    return jnp.where(t > 0, t + 1.0, jnp.exp(t)) + 1e-6


def _sigmoid(t):
    return 1.0 / (1.0 + jnp.exp(-t))


def _matvec_chain(w_refs, col_ref, n_rows, n_cols, live, width, prev):
    rep = width // BLK
    outs = [[] for _ in w_refs]
    for c0 in range(0, n_cols, width):
        for w_ref, out in zip(w_refs, outs):
            def step(i, acc, w_ref=w_ref):
                r0 = pl.multiple_of(i * 8, 8)
                col = col_ref[pl.ds(r0, 8), :]
                w = w_ref[pl.ds(r0, 8), c0:c0 + width].astype(f32)
                return acc + w * jnp.concatenate([col] * rep, axis=1)
            link = _link(live, prev)
            acc = lax.fori_loop(0, n_rows // 8, step, jnp.concatenate([link] * rep, axis=1),
                                unroll=True)
            out.append(acc)
            prev = acc[:, 0:BLK]
            for h in range(1, rep):
                prev = prev + acc[:, h * BLK:(h + 1) * BLK]
    return [jnp.concatenate(o, axis=1) for o in outs], prev


SCRATCH = dict(
    x_v=((S, D), bf16), wq_v=((D, D), bf16), wk_v=((D, D), bf16), wv_v=((D, D), bf16),
    wo_v=((D, D), bf16), wg_v=((D, F), bf16), wu_v=((D, F), bf16), wd_v=((F, D), bf16),
    wr_v=((D,), bf16), gw_v=((D,), bf16),
    xs_v=((5 * HS // 2, HD), u32),
    wks_v=((5 * HD // 2, HD), u32),
    wqs_v=((7 * HD // 2, HD), u32),
    pks_v=((7 * HD // 2, HS), u32),
    g_v=((D // 2, D), u32),
    ms_v=((7 * HD // 2, HD), u32),
    ps_v=((7 * HS // 2, HD), u32),
    out_v=((S, D), bf16),
    gate_v=((S, BLK), f32),
    zc_v=((D, BLK), f32),
    xc_v=((D, BLK), f32),
    hc_v=((F, BLK), f32),
    ck_v=((4, R, HD), f32),
    cq_v=((4, HD, R), f32),
    cg_v=((2, HD, HD), f32),
    wb_v=((2, 8, D), f32),
    c0_v=((2 * R, D), f32),
    gu_v=((2, 8, F), f32),
    sel_v=((2, 8, BLK), f32),
)


OUT_ORDER = tuple(tuple(half * HS + r0 for r0 in range(0, HS, R) for half in ((1, 0), (0, 1))[col])
                  for col in range(2))


N_LAG = 2 * (NP - 1)


def _blocks(v, start_out, state):
    x_v, wk_v, wq_v = v["x_v"], v["wk_v"], v["wq_v"]
    xs_v, ps_v = (_Packed(v[k], HS) for k in ("xs_v", "ps_v"))
    wks_v, wqs_v, pks_v, ms_v = (_Packed(v[k], HD) for k in ("wks_v", "wqs_v", "pks_v", "ms_v"))
    ck_v, cq_v, cg_v, c0_v, gu_v, sel_v = (v[k] for k in (
        "ck_v", "cq_v", "cg_v", "c0_v", "gu_v", "sel_v"))
    g_v, gate_v, zc_v, xc_v, hc_v, out_v = (v[k] for k in (
        "g_v", "gate_v", "zc_v", "xc_v", "hc_v", "out_v"))
    zero = jnp.zeros((8, BLK), f32)

    def get_live():
        words = pltpu.bitcast(x_v[0:16, 0:BLK], jnp.int32)
        return lax.shift_right_arithmetic(words, 31) >= -1

    def x_form(f, r0, n):
        if f == 5:
            return x_v[r0:r0 + n, 0:HD]
        if f == 6:
            return x_v[HS + r0:HS + r0 + n, HD:D]
        return xs_v.get(f, r0, n)

    def sel_idx():
        return state["idx"]

    def wk_form(f):
        if f == 5:
            return wk_v[0:HD, 0:HD]
        if f == 6:
            return wk_v[HD:D, HD:D]
        return wks_v.get(f)

    def free_forms(src, dst, r0, n, half_rows, f):
        blocks = [src[rr:rr + n, cc:cc + HD].astype(f32)
                  for rr in (r0, half_rows + r0) for cc in (0, HD)]
        dst.put(_forms(*blocks)[f], f, r0)

    def make_wq_forms(live, pad):
        prev = zero
        for r in range(0, HD, BLK):
            for c in range(0, HD, 2 * BLK):
                tiles = [wq_v[rr:rr + 2 * BLK, cc:cc + BLK].T.astype(f32)
                         for rr, cc in ((c, r), (c, HD + r), (HD + c, r), (HD + c, HD + r))]
                for c1 in range(0, 2 * BLK, BLK):
                    rows = []
                    for s0 in range(0, BLK, 8):
                        fs, prev = _chained_forms([t[s0:s0 + 8, c1:c1 + BLK] for t in tiles],
                                                  live, prev, pad)
                        rows.append(fs)
                    for f in range(7):
                        wqs_v.put(jnp.concatenate([fs[f] for fs in rows], axis=0), f, r, c + c1)
        return prev

    def anchored(prod, i, ref, f, live, prev):
        def wrapped(m):
            if m == i:
                link = jnp.concatenate([_link(live, prev)] * 2, axis=0)
                ref.put(ref.get(f, 0, 16, 0, BLK).astype(f32) + link, f)
            return prod(m)
        return wrapped

    def last_rows(t):
        out = []
        for r in range(BLK, t.shape[0] + 1, BLK):
            last = t[r - 16:r, :].astype(f32)[8:16]
            out += [last[:, c:c + BLK] for c in range(0, t.shape[1], BLK)]
        return _tree_sum(out)

    def k_post(c, col, half):
        return _phi(c)

    done = []

    def k_epi(j, p, z):
        p11, p12, p21, p22 = p
        zs = jnp.concatenate([jnp.sum((p11 + p21).reshape(R // 8, 8, HD), axis=0),
                              jnp.sum((p12 + p22).reshape(R // 8, 8, HD), axis=0)], axis=1)
        fs = _forms(p11, p21, p12, p22)
        for f in (5, 2, 6, 0, 1, 4, 3):
            t = fs[f].astype(bf16).T
            pks_v.put(t, f, 0, j * R)
            done.append(last_rows(t))
        return zs if z is None else z + zs

    def k_prod(j):
        return lambda i: _dot(x_form(A_FORM[i], j * R, R), wk_form(B_FORM[i]))

    def g_prod(i, k0=0, k1=HS):
        return _dot(pks_v.get(A_FORM[i], c0=k0, c1=k1), x_form(B_FORM[i], k0, k1 - k0))

    def q_prod(j):
        return lambda i: _dot(wqs_v.get(B_FORM[i]), x_form(A_FORM[i], j * R, R), _NT)

    def q_post(c, col, half):
        pq = _phi(c)
        zc = jnp.tile(zc_v[col * HD:(col + 1) * HD, :], (1, R // BLK))
        w = (pq * zc).reshape(H // 2, DH // 8, 8, R)
        eps = jnp.where(lax.broadcasted_iota(jnp.int32, (8, R), 0) == 0, 1e-6, 0.0)
        part = ((w[:, 0] + eps) + w[:, 1]) + w[:, 2] + w[:, 3]
        den = jnp.sum(part, axis=1, keepdims=True)
        return (pq.reshape(H // 2, DH, R) * _recip(den)).reshape(HD, R)

    def q_epi(j, p):
        fs = _forms(*p)
        ends = []
        for f in range(7):
            t = fs[f].astype(bf16).T
            ps_v.put(t, f, j * R)
            ends.append(last_rows(t))
        return _tree_sum(ends)

    def ramp(i):
        k0, n = K_CHUNKS[i]

        def run():
            xx = jnp.concatenate([x_v[0:R, k0:k0 + n], x_v[HS:HS + R, k0:k0 + n]], axis=0)
            c = _dot(xx, wk_v[k0:k0 + n, :])
            c0_v[...] = c0_v[...] + c if i else c
        return run

    def b4():
        sep_forms(1, (2, 1, 0, 4, 3))
        for f in (0, 1, 2):
            free_forms(wk_v, wks_v, 0, HD, HD, f)
        head = _strassen_head2(k_prod(1))
        for i in range(4):
            ck_v[i] = head[i]

    def sep_forms(j, which):
        for f in which:
            free_forms(x_v, xs_v, j * R, R, HS, f)

    def router(live, prev):
        wr_ref, gw_ref = v["wb_v"].at[0], v["wb_v"].at[1]
        v["wb_v"][0] = jnp.broadcast_to(v["wr_v"][...].astype(f32).reshape(1, D), (8, D))
        v["wb_v"][1] = jnp.broadcast_to(v["gw_v"][...].astype(f32).reshape(1, D), (8, D))
        rows, ends = [], []
        for t in range(S // BLK):
            accs = [[], []]
            for r in range(t * BLK, (t + 1) * BLK, 8):
                ar = ag = _link(live, prev)
                for c in range(0, D, 2 * BLK):
                    xx = x_v[r:r + 8, c:c + 2 * BLK].astype(f32)
                    for h in range(2):
                        cs = slice(c + h * BLK, c + (h + 1) * BLK)
                        xh = xx[:, h * BLK:(h + 1) * BLK]
                        ar = ar + xh * wr_ref[:, cs]
                for c in range(0, D, 2 * BLK):
                    xx = x_v[r:r + 8, c:c + 2 * BLK].astype(f32)
                    for h in range(2):
                        cs = slice(c + h * BLK, c + (h + 1) * BLK)
                        xh = xx[:, h * BLK:(h + 1) * BLK]
                        ag = ag + xh * gw_ref[:, cs]
                prev = ar + ag
                accs[0].append(ar)
                accs[1].append(ag)
            sums = [jnp.sum(jnp.concatenate(a, axis=0).T, axis=0, keepdims=True) for a in accs]
            rows.append(sums[0])
            gate = jnp.broadcast_to(_sigmoid(sums[1]), (BLK, BLK)).T
            gate_v[t * BLK:(t + 1) * BLK, :] = gate
            ends.append(gate[BLK - 8:])
        r = jnp.concatenate(rows, axis=1).astype(bf16).astype(f32)
        r_max = jnp.max(r, axis=1, keepdims=True)
        lane = lax.broadcasted_iota(jnp.int32, (1, S), 1)
        idx_v = jnp.min(jnp.where(r == r_max, lane, S), axis=1, keepdims=True)
        idx_v = jnp.clip(idx_v, 0, S - 1)
        sel_v[0] = jnp.broadcast_to(_sigmoid(r_max), (8, BLK))
        sel_v[1] = jnp.broadcast_to(idx_v.astype(f32), (8, BLK))
        idx = idx_v[0, 0]
        state["idx"] = idx
        base = pl.multiple_of((idx // 16) * 16, 16)
        slab = x_v[pl.ds(base, 16), :].astype(f32)
        rid = lax.broadcasted_iota(jnp.int32, (16, D), 0)
        x_sel = jnp.sum(jnp.where(rid == idx - base, slab, 0.0), axis=0, keepdims=True)
        xc = jnp.broadcast_to(x_sel, (BLK, D)).T
        xc_v[...] = xc
        return last_slabs(xc) + _tree_sum(ends)

    def last_slabs(a):
        n = a.shape[0] // BLK
        return jnp.sum(a.reshape(n, BLK // 8, 8, BLK)[:, BLK // 8 - 1], axis=0)

    def b5():
        live = get_live()
        for f in (4, 3):
            free_forms(wk_v, wks_v, 0, HD, HD, f)
        z = k_epi(1, _strassen_tail2(k_prod(1), k_post, [ck_v[i] for i in range(4)]), None)
        z = k_epi(0, [_phi(c0_v[r:r + R, c:c + HD]) for r in (0, R) for c in (0, HD)], z)
        sep_forms(2, (2, 1, 0, 4, 3))
        z = k_epi(2, _strassen(k_prod(2), k_post), z)
        sep_forms(3, (2, 1, 0, 4, 3))
        z = k_epi(3, _strassen(k_prod(3), k_post), z)
        z = jnp.sum(z, axis=0, keepdims=True)
        zc = jnp.broadcast_to(z, (BLK, D)).T
        zc_v[...] = zc
        sep_forms(0, (4, 3, 0))
        end = router(live, _tree_sum(done) + last_slabs(zc))

        m3 = g_prod(2, R, HS - R) + g_prod(2, 0, R) + g_prod(2, HS - R, HS)
        m5 = g_prod(4)
        g_v[0:HD // 2, HD:D] = _pk(m3 + m5)
        m4 = g_prod(3)
        m2 = g_prod(1)
        g_v[HD // 2:D // 2, 0:HD] = _pk(m2 + m4)
        m1 = g_prod(0)
        link = jnp.concatenate([_link(live, end)] * (HD // BLK), axis=1)
        m1 = jnp.concatenate([m1[:HD - 8], m1[HD - 8:] + link], axis=0)
        cg_v[0] = m1 + (m4 - m5)
        cg_v[1] = m1 + (m3 - m2)

    def b6():
        live = get_live()
        sep_forms(0, (1, 2))
        g_v[0:HD // 2, 0:HD] = _pk(cg_v[0] + g_prod(6, R, HS) + g_prod(6, 0, R))
        g_v[HD // 2:D // 2, HD:D] = _pk(cg_v[1] + g_prod(5))
        end = make_wq_forms(live, 3)
        (gg, uu), end = _matvec_chain((v["wg_v"], v["wu_v"]), xc_v, D, F, live, 2 * BLK, end)
        gu_v[0] = gg
        gu_v[1] = uu
        head = _strassen_head(anchored(q_prod(0), 0, wqs_v, B_FORM[0], live, end), q_post)
        for i in range(4):
            cq_v[i] = head[i]

    def a_prod(j):
        return lambda m: _dot(ps_v.get(A_FORM[m], j * R, R), ms_v.get(B_FORM[m]))

    def a_post(j, y=None):
        def post(a, col, half):
            rr = j * R + half * HS
            cs = slice(col * HD, (col + 1) * HD)
            g = jnp.tile(gate_v[rr:rr + R, :], (1, HD // BLK))
            b = x_v[rr:rr + R, cs].astype(f32)
            if y is not None:
                rows = lax.broadcasted_iota(jnp.int32, (R, HD), 0)
                b = b + jnp.where(rows == sel_idx() - rr, y[:, cs], 0.0)
            out_v[rr:rr + R, cs] = (g * a + (1.0 - g) * b).astype(bf16)
            k = OUT_ORDER[col].index(rr)
            if k:
                start_out(col, k)
        return post

    def b7():
        live = get_live()
        sel_idx()
        gg = jnp.sum(gu_v[0], axis=0, keepdims=True)
        uu = jnp.sum(gu_v[1], axis=0, keepdims=True)
        hh = gg * _sigmoid(gg) * uu
        hc = jnp.broadcast_to(hh, (BLK, F)).T
        hc_v[...] = hc
        p = _strassen_tail(q_prod(0), q_post, [cq_v[i] for i in range(4)])
        ri = lax.broadcasted_iota(jnp.int32, (BLK, BLK), 0) // DH
        ci = lax.broadcasted_iota(jnp.int32, (BLK, BLK), 1) // DH
        diag = ri == ci
        kvs = []
        for j in range(NB):
            sl = slice(j * BLK, (j + 1) * BLK)
            kv = _dot(_unpk(g_v[j * BLK // 2:(j + 1) * BLK // 2, :]), v["wv_v"][:, sl])
            kvs.append(jnp.where(diag, kv, 0.0).astype(bf16))
        q_epi(0, p)
        for j in range(NB // 2):
            j2 = j + NB // 2
            mu = _dot(kvs[j], v["wo_v"][j * BLK:(j + 1) * BLK, :])
            ml = _dot(kvs[j2], v["wo_v"][j2 * BLK:(j2 + 1) * BLK, :])
            fs = _forms(mu[:, :HD], mu[:, HD:], ml[:, :HD], ml[:, HD:])
            for f in range(7):
                ms_v.put(fs[f], f, j * BLK)
        ends = [q_epi(1, _strassen(anchored(q_prod(1), 2, wqs_v, B_FORM[2], live, last_slabs(hc)),
                                   q_post)),
                q_epi(2, _strassen(q_prod(2), q_post)),
                q_epi(3, _strassen(q_prod(3), q_post))]
        prod = anchored(a_prod(0), 0, ms_v, B_FORM[0], live, _tree_sum(ends))
        head = _strassen_head(prod, a_post(0))
        ck_v[0] = head[2]
        ck_v[1] = head[3]

    def b8():
        live = get_live()
        idx = sel_idx()
        (yy,), _ = _matvec_chain((v["wd_v"],), hc_v, F, D, live, BLK, zero)
        y = jnp.sum(yy, axis=0, keepdims=True) * sel_v[0, 0:1, 0:1]

        _strassen_tail(a_prod(0), a_post(0), (None, None, ck_v[0], ck_v[1]))
        for j in range(1, NP - 1):
            _strassen(a_prod(j), a_post(j))
        rid = lax.broadcasted_iota(jnp.int32, (16, HD), 0)
        for col in range(2):
            cs = slice(col * HD, (col + 1) * HD)
            base = jnp.where(idx % HS < HS - R, (idx // 16) * 16, OUT_ORDER[col][N_LAG - 1])
            base = pl.multiple_of(base, 16)
            g = jnp.tile(gate_v[pl.ds(base, 16), :], (1, HD // BLK))
            upd = jnp.where(rid == idx - base, (1.0 - g) * y[:, cs], 0.0)
            out_v[pl.ds(base, 16), cs] = (out_v[pl.ds(base, 16), cs].astype(f32) + upd).astype(bf16)
            start_out(col, 0)
        _strassen(a_prod(NP - 1), a_post(NP - 1, y))

    return [ramp(i) for i in range(NK)] + [b4, b5, b6, b7, b8]


def _start_out(src, dst, sem, idx, col, k):
    order = OUT_ORDER[col]
    widths = [(col * HD, HD)]
    if k >= N_LAG:
        r0 = order[k]
        if col == 1 and k == len(order) - 1:
            widths = [(c, BLK) for c in range(HD, D, BLK)]
    else:
        blk = (idx // R) * R
        n = k if k else N_LAG - 1
        seen = functools.reduce(jnp.logical_or, [blk == r for r in order[:n]])
        r0 = jnp.where(seen, order[k], order[k - 1]) if k else jnp.where(seen, blk, order[N_LAG - 1])
        r0 = pl.multiple_of(r0, R)
    for c, n in widths:
        pltpu.make_async_copy(src.at[pl.ds(r0, R), pl.ds(c, n)], dst.at[pl.ds(r0, R), pl.ds(c, n)],
                              sem).start()


def _kernel(x_hbm, wqkv_hbm, wo_hbm, wr_hbm, wg_hbm, wu_hbm, wd_hbm, gw_hbm,
            out_hbm, *scratch):
    v = dict(zip(SCRATCH, scratch))
    sem_hi, sem_lo, sem_o = scratch[len(SCRATCH):]

    def x_copy(j, half):
        r0 = half * HS + j * R
        return pltpu.make_async_copy(x_hbm.at[0, pl.ds(r0, R), :], v["x_v"].at[pl.ds(r0, R), :],
                                     sem_hi.at[NK + min(j - 1, 1)])

    def ramp_copies(i):
        k0, n = K_CHUNKS[i]
        return [pltpu.make_async_copy(x_hbm.at[0, pl.ds(r0, R), pl.ds(k0, n)],
                                      v["x_v"].at[pl.ds(r0, R), pl.ds(k0, n)], sem_hi.at[i])
                for r0 in (0, HS)] + [
            pltpu.make_async_copy(wqkv_hbm.at[pl.ds(k0, n), pl.ds(D, D)],
                                  v["wk_v"].at[pl.ds(k0, n), :], sem_hi.at[i])]

    cp_wq = pltpu.make_async_copy(wqkv_hbm.at[:, pl.ds(0, D)], v["wq_v"], sem_lo.at[1])
    cp_wv = pltpu.make_async_copy(wqkv_hbm.at[:, pl.ds(2 * D, D)], v["wv_v"], sem_lo.at[2])
    cp_wo = pltpu.make_async_copy(wo_hbm, v["wo_v"], sem_lo.at[2])
    cp_wg = pltpu.make_async_copy(wg_hbm, v["wg_v"], sem_lo.at[1])
    cp_wu = pltpu.make_async_copy(wu_hbm, v["wu_v"], sem_lo.at[1])
    cp_wd = pltpu.make_async_copy(wd_hbm, v["wd_v"], sem_lo.at[3])
    cp_wr = pltpu.make_async_copy(wr_hbm, v["wr_v"], sem_lo.at[0])
    cp_gw = pltpu.make_async_copy(gw_hbm, v["gw_v"], sem_lo.at[0])

    state = {}

    waits = [ramp_copies(i) for i in range(NK)] + [
        [x_copy(1, 0), x_copy(1, 1)],
        [x_copy(j, h) for j in range(2, NP) for h in range(2)] + [cp_wr, cp_gw],
        [cp_wg, cp_wu, cp_wq],
        [cp_wv, cp_wo],
        [cp_wd],
    ]
    for cp in sum(waits[:NK + 1], []) + waits[NK + 1][:-2]:
        cp.start()
    blocks = _blocks(v, lambda col, k: _start_out(v["out_v"], out_hbm.at[0], sem_o, state["idx"], col, k),
                     state)
    for n, (ws, blk) in enumerate(zip(waits, blocks)):
        for cp in ws:
            cp.wait()
        if n == 3:
            for cp in (cp_wr, cp_gw, cp_wg, cp_wu, cp_wq, cp_wv, cp_wo, cp_wd):
                cp.start(priority=1)
        blk()
    pltpu.make_async_copy(v["out_v"], out_hbm.at[0], sem_o).wait()


@jax.jit
def pallas_gated_mix__linear_attn_block__moe_arch_mod__prompt_kernel(
    A_x: jax.Array,
    A_wqkv: jax.Array,
    A_wo: jax.Array,
    B_x: jax.Array,
    B_w_r: jax.Array,
    B_w_gate: jax.Array,
    B_w_up: jax.Array,
    B_w_down: jax.Array,
    gate_w: jax.Array,
):
    del B_x
    any_spec = pl.BlockSpec(memory_space=pl.ANY)
    scratch = [pltpu.VMEM(*s) for s in SCRATCH.values()] + [
        pltpu.SemaphoreType.DMA((NK + 2,)),
        pltpu.SemaphoreType.DMA((4,)),
        pltpu.SemaphoreType.DMA(()),
    ]
    return pl.pallas_call(
        _kernel,
        out_shape=jax.ShapeDtypeStruct((1, S, D), bf16),
        in_specs=[any_spec] * 8,
        out_specs=any_spec,
        scratch_shapes=scratch,
        compiler_params=pltpu.CompilerParams(vmem_limit_bytes=120 * 1024 * 1024,
                                             disable_semaphore_checks=True),
    )(A_x, A_wqkv, A_wo, B_w_r, B_w_gate, B_w_up, B_w_down, gate_w)
```

```python
import functools
import jax
import jax.numpy as jnp
from jax import lax
import jax.experimental.pallas as pl
import jax.experimental.pallas.tpu as pltpu

S = 2048
D = 1024
F = 3584
H = 32
DH = D // H
HS = S // 2
HD = D // 2
HQ = D // 4
R = 256
NP = HS // R
BLK = 128
NB = D // BLK
K_CHUNKS = ((0, 128), (128, 128), (256, 256), (512, 256), (768, 256))
NK = len(K_CHUNKS)

_NN = (((1,), (0,)), ((), ()))
_NT = (((1,), (1,)), ((), ()))
_TN = (((0,), (0,)), ((), ()))
f32 = jnp.float32
bf16 = jnp.bfloat16
u32 = jnp.uint32


A_FORM = (0, 1, 5, 6, 2, 3, 4)
B_FORM = (0, 5, 4, 3, 6, 2, 1)


G_ORDER = (3, 4, 0, 1)


def _forms(b11, b12, b21, b22):
    return (b11 + b22, b21 + b22, b11 + b12, b21 - b11, b12 - b22, b11, b22)


def _strassen_head(prod, post):
    m3 = prod(2)
    m4 = prod(3)
    m5 = prod(4)
    p12 = post(m3 + m5, 1, 0)
    m2 = prod(1)
    p21 = post(m2 + m4, 0, 1)
    m1 = prod(0)
    return p12, p21, (m1 + m4) - m5, (m1 - m2) + m3


def _strassen_tail(prod, post, head):
    p12, p21, t11, t22 = head
    p11 = post(t11 + prod(6), 0, 0)
    p22 = post(t22 + prod(5), 1, 1)
    return p11, p12, p21, p22


def _strassen_head2(prod):
    m5 = prod(4)
    m2 = prod(1)
    m1 = prod(0)
    t11 = (m1 - m5) + prod(6)
    t22 = (m1 - m2) + prod(5)
    return m5, m2, t11, t22


def _strassen_tail2(prod, post, head):
    m5, m2, t11, t22 = head
    m3 = prod(2)
    p12 = post(m3 + m5, 1, 0)
    p22 = post(t22 + m3, 1, 1)
    m4 = prod(3)
    p21 = post(m2 + m4, 0, 1)
    p11 = post(t11 + m4, 0, 0)
    return p11, p12, p21, p22


def _strassen(prod, post):
    return _strassen_tail(prod, post, _strassen_head(prod, post))


def _pk(a):
    return pltpu.bitcast(a.astype(bf16), u32)


def _unpk(a):
    return pltpu.bitcast(a, bf16)


class _Packed:
    def __init__(self, ref, rows):
        self.ref, self.rows = ref, rows

    def _idx(self, f, r0, n, c0, c1):
        n = self.rows - r0 if n is None else n
        a = (f * self.rows + r0) // 2
        return slice(a, a + n // 2), slice(c0, c1)

    def get(self, f, r0=0, n=None, c0=None, c1=None):
        return _unpk(self.ref[self._idx(f, r0, n, c0, c1)])

    def put(self, val, f, r0=0, c0=0):
        self.ref[self._idx(f, r0, val.shape[0], c0, c0 + val.shape[1])] = _pk(val)


def _link(live, prev):
    return jnp.where(live, 0.0, prev)


def _chained_forms(blocks, live, prev, pad):
    b11, b12, b21, b22 = blocks
    b11 = b11 + _link(live, prev)
    s1112 = b11 + b12
    s2122 = b21 + b22
    prev = s1112 + s2122
    for _ in range(pad):
        prev = prev + s2122
    return (b11 + b22, s2122, s1112, b21 - b11, b12 - b22, b11, b22), prev


def _recip(d):
    r = pltpu.bitcast(jnp.int32(0x7EF311C3) - pltpu.bitcast(d, jnp.int32), f32)
    r = r * (2.00130856 - d * r)
    return r * (2.00000084 - d * r)


def _tree_sum(vals):
    while len(vals) > 1:
        vals = [sum(vals[i + 1:i + 2], vals[i]) for i in range(0, len(vals), 2)]
    return vals[0]


def _dot(a, b, dims=_NN):
    return lax.dot_general(a, b, dims, preferred_element_type=f32)


def _phi(t):
    return jnp.where(t > 0, t + 1.0, jnp.exp(t)) + 1e-6


def _sigmoid(t):
    return 1.0 / (1.0 + jnp.exp(-t))


def _matvec_chain(w_refs, col_ref, n_rows, n_cols, live, width, prev):
    rep = width // BLK
    outs = [[] for _ in w_refs]
    for c0 in range(0, n_cols, width):
        for w_ref, out in zip(w_refs, outs):
            def step(i, acc, w_ref=w_ref):
                r0 = pl.multiple_of(i * 8, 8)
                col = col_ref[pl.ds(r0, 8), :]
                w = w_ref[pl.ds(r0, 8), c0:c0 + width].astype(f32)
                return acc + w * jnp.concatenate([col] * rep, axis=1)
            link = _link(live, prev)
            acc = lax.fori_loop(0, n_rows // 8, step, jnp.concatenate([link] * rep, axis=1),
                                unroll=True)
            out.append(acc)
            prev = acc[:, 0:BLK]
            for h in range(1, rep):
                prev = prev + acc[:, h * BLK:(h + 1) * BLK]
    return [jnp.concatenate(o, axis=1) for o in outs], prev


SCRATCH = dict(
    x_v=((S, D), bf16), wq_v=((D, D), bf16), wk_v=((D, D), bf16), wv_v=((D, D), bf16),
    wo_v=((D, D), bf16), wg_v=((D, F), bf16), wu_v=((D, F), bf16), wd_v=((F, D), bf16),
    wr_v=((D,), bf16), gw_v=((D,), bf16),
    xs_v=((5 * HS // 2, HD), u32),
    wks_v=((5 * HD // 2, HD), u32),
    wqs_v=((7 * HD // 2, HD), u32),
    pks_v=((7 * HD // 2, HS), u32),
    g_v=((D // 2, D), u32),
    ga_v=((6 * 5 * HQ // 2, HS // 2), u32),
    gb_v=((6 * 5 * HS // 4, HQ), u32),
    ms_v=((7 * HD // 2, HD), u32),
    ps_v=((7 * HS // 2, HD), u32),
    out_v=((S, D), bf16),
    gate_v=((S, BLK), f32),
    zc_v=((D, BLK), f32),
    xc_v=((D, BLK), f32),
    hc_v=((F, BLK), f32),
    ck_v=((4, R, HD), f32),
    cq_v=((4, HD, R), f32),
    cg_v=((2, HD, HD), f32),
    wb_v=((2, 8, D), f32),
    c0_v=((2 * R, D), f32),
    gu_v=((2, 8, F), f32),
    sel_v=((2, 8, BLK), f32),
)


A_GROUPS = ((0, 1), (2, 3))
OUT_ORDER = tuple(tuple(half * HS + j * R for grp in A_GROUPS for half in ((1, 0), (0, 1))[col]
                        for j in grp) for col in range(2))


N_LAG = 2 * A_GROUPS[-1][0]


def _blocks(v, start_out, state):
    x_v, wk_v, wq_v = v["x_v"], v["wk_v"], v["wq_v"]
    xs_v, ps_v = (_Packed(v[k], HS) for k in ("xs_v", "ps_v"))
    wks_v, wqs_v, pks_v, ms_v = (_Packed(v[k], HD) for k in ("wks_v", "wqs_v", "pks_v", "ms_v"))
    ck_v, cq_v, cg_v, c0_v, gu_v, sel_v = (v[k] for k in (
        "ck_v", "cq_v", "cg_v", "c0_v", "gu_v", "sel_v"))
    g_v, gate_v, zc_v, xc_v, hc_v, out_v = (v[k] for k in (
        "g_v", "gate_v", "zc_v", "xc_v", "hc_v", "out_v"))
    zero = jnp.zeros((8, BLK), f32)

    def get_live():
        words = pltpu.bitcast(x_v[0:16, 0:BLK], jnp.int32)
        return lax.shift_right_arithmetic(words, 31) >= -1

    def x_form(f, r0, n, c0=0, c1=HD):
        if f == 5:
            return x_v[r0:r0 + n, c0:c1]
        if f == 6:
            return x_v[HS + r0:HS + r0 + n, HD + c0:HD + c1]
        return xs_v.get(f, r0, n, c0, c1)

    def sel_idx():
        return state["idx"]

    def wk_form(f):
        if f == 5:
            return wk_v[0:HD, 0:HD]
        if f == 6:
            return wk_v[HD:D, HD:D]
        return wks_v.get(f)

    def free_forms(src, dst, r0, n, half_rows, f):
        blocks = [src[rr:rr + n, cc:cc + HD].astype(f32)
                  for rr in (r0, half_rows + r0) for cc in (0, HD)]
        dst.put(_forms(*blocks)[f], f, r0)

    def make_wq_forms(live, pad):
        prev = zero
        for r in range(0, HD, BLK):
            for c in range(0, HD, 2 * BLK):
                tiles = [wq_v[rr:rr + 2 * BLK, cc:cc + BLK].T.astype(f32)
                         for rr, cc in ((c, r), (c, HD + r), (HD + c, r), (HD + c, HD + r))]
                for c1 in range(0, 2 * BLK, BLK):
                    rows = []
                    for s0 in range(0, BLK, 8):
                        fs, prev = _chained_forms([t[s0:s0 + 8, c1:c1 + BLK] for t in tiles],
                                                  live, prev, pad)
                        rows.append(fs)
                    for f in range(7):
                        wqs_v.put(jnp.concatenate([fs[f] for fs in rows], axis=0), f, r, c + c1)
        return prev

    def anchored(prod, i, ref, f, live, prev):
        def wrapped(m):
            if m == i:
                link = jnp.concatenate([_link(live, prev)] * 2, axis=0)
                ref.put(ref.get(f, 0, 16, 0, BLK).astype(f32) + link, f)
            return prod(m)
        return wrapped

    def last_rows(t):
        out = []
        for r in range(BLK, t.shape[0] + 1, BLK):
            last = t[r - 16:r, :].astype(f32)[8:16]
            out += [last[:, c:c + BLK] for c in range(0, t.shape[1], BLK)]
        return _tree_sum(out)

    def k_post(c, col, half):
        return _phi(c)

    done = []

    def k_epi(j, p, z):
        p11, p12, p21, p22 = p
        zs = jnp.concatenate([jnp.sum((p11 + p21).reshape(R // 8, 8, HD), axis=0),
                              jnp.sum((p12 + p22).reshape(R // 8, 8, HD), axis=0)], axis=1)
        fs = _forms(p11, p21, p12, p22)
        for f in [5] + [A_FORM[i] for i in G_ORDER] + [4, 3]:
            t = fs[f].astype(bf16).T
            pks_v.put(t, f, 0, j * R)
            done.append(last_rows(t))
        return zs if z is None else z + zs

    def k_prod(j):
        return lambda i: _dot(x_form(A_FORM[i], j * R, R), wk_form(B_FORM[i]))

    def g_prod(i, k0=0, k1=HS):
        return _dot(pks_v.get(A_FORM[i], c0=k0, c1=k1), x_form(B_FORM[i], k0, k1 - k0))

    ga_v, gb_v = _Packed(v["ga_v"], HQ), _Packed(v["gb_v"], HS // 2)

    def g_prod2(i, slot):
        kh = HS // 2

        def form(blk, dst, f):
            if f >= 5:
                return blk(f - 5, f - 5)
            blocks = [blk(r, c).astype(f32) for r in range(2) for c in range(2)]
            dst.put(_forms(*blocks)[f], 5 * slot + f)
            return dst.get(5 * slot + f, 0, dst.rows)

        def a_blk(r, c):
            return pks_v.get(A_FORM[i], r * HQ, HQ, c * kh, (c + 1) * kh)

        def b_blk(r, c):
            return x_form(B_FORM[i], r * kh, kh, c * HQ, (c + 1) * HQ)

        p11, p12, p21, p22 = _strassen(
            lambda m: _dot(form(a_blk, ga_v, A_FORM[m]), form(b_blk, gb_v, B_FORM[m])),
            lambda c, col, half: c)
        return jnp.concatenate([jnp.concatenate([p11, p12], axis=1),
                                jnp.concatenate([p21, p22], axis=1)], axis=0)

    gs_v = _Packed(v["gb_v"], HQ)

    def second_level(m, l_blk, r_blk, dims, plain, kept=()):
        if m in plain:
            ls, rs = ([[blk(r, c) for c in range(2)] for r in range(2)] for blk in (l_blk, r_blk))
            ax = 1 if dims == _NN else 0
            left = jnp.concatenate([jnp.concatenate(row, axis=1) for row in ls], axis=0)
            right = jnp.concatenate([jnp.concatenate(row, axis=ax) for row in rs], axis=1 - ax)
            return _dot(left, right, dims)

        def form(blk, side, f):
            if f >= 5:
                return blk(f - 5, f - 5)
            n = 5 * m + f
            if side and m in kept:
                return gs_v.get(n, 0, HQ)
            val = _forms(*[blk(r, c).astype(f32) for r in range(2) for c in range(2)])[f]
            if side:
                gs_v.put(val, n)
                return gs_v.get(n, 0, HQ)
            ga_v.put(val, n // 2, 0, (n % 2) * HQ)
            return ga_v.get(n // 2, 0, HQ, (n % 2) * HQ, (n % 2 + 1) * HQ)

        p11, p12, p21, p22 = _strassen(
            lambda i: _dot(form(l_blk, 0, A_FORM[i]), form(r_blk, 1, B_FORM[i]), dims),
            lambda c, col, half: c)
        return jnp.concatenate([jnp.concatenate([p11, p12], axis=1),
                                jnp.concatenate([p21, p22], axis=1)], axis=0)

    def a_prod2(j):
        first = (0, 5, 6)
        plain = () if j else first
        kept = [m for m in range(7) if m not in first] if j else ()
        return lambda m: second_level(
            m, lambda r, c: ps_v.get(A_FORM[m], (j + r) * R, R, c * HQ, (c + 1) * HQ),
            lambda r, c: ms_v.get(B_FORM[m], r * HQ, HQ, c * HQ, (c + 1) * HQ), _NN, plain, kept)

    def q_prod(j):
        return lambda i: _dot(wqs_v.get(B_FORM[i]), x_form(A_FORM[i], j * R, R), _NT)

    def q_post(c, col, half):
        pq = _phi(c)
        zc = jnp.tile(zc_v[col * HD:(col + 1) * HD, :], (1, R // BLK))
        w = (pq * zc).reshape(H // 2, DH // 8, 8, R)
        eps = jnp.where(lax.broadcasted_iota(jnp.int32, (8, R), 0) == 0, 1e-6, 0.0)
        part = ((w[:, 0] + eps) + w[:, 1]) + w[:, 2] + w[:, 3]
        den = jnp.sum(part, axis=1, keepdims=True)
        return (pq.reshape(H // 2, DH, R) * _recip(den)).reshape(HD, R)

    def q_epi(j, p):
        fs = _forms(*p)
        ends = []
        for f in range(7):
            t = fs[f].astype(bf16).T
            ps_v.put(t, f, j * R)
            ends.append(last_rows(t))
        return _tree_sum(ends)

    def ramp(i):
        k0, n = K_CHUNKS[i]

        def run():
            xx = jnp.concatenate([x_v[0:R, k0:k0 + n], x_v[HS:HS + R, k0:k0 + n]], axis=0)
            c = _dot(xx, wk_v[k0:k0 + n, :])
            c0_v[...] = c0_v[...] + c if i else c
        return run

    def b4():
        sep_forms(1, (2, 1, 0, 4, 3))
        for f in (0, 1, 2):
            free_forms(wk_v, wks_v, 0, HD, HD, f)
        head = _strassen_head2(k_prod(1))
        for i in range(4):
            ck_v[i] = head[i]

    def sep_forms(j, which):
        for f in which:
            free_forms(x_v, xs_v, j * R, R, HS, f)

    def router(live, prev):
        wr_ref, gw_ref = v["wb_v"].at[0], v["wb_v"].at[1]
        v["wb_v"][0] = jnp.broadcast_to(v["wr_v"][...].astype(f32).reshape(1, D), (8, D))
        v["wb_v"][1] = jnp.broadcast_to(v["gw_v"][...].astype(f32).reshape(1, D), (8, D))
        rows, ends = [], []
        for t in range(S // BLK):
            accs = [[], []]
            for r in range(t * BLK, (t + 1) * BLK, 8):
                ar = ag = _link(live, prev)
                for c in range(0, D, 2 * BLK):
                    xx = x_v[r:r + 8, c:c + 2 * BLK].astype(f32)
                    for h in range(2):
                        cs = slice(c + h * BLK, c + (h + 1) * BLK)
                        xh = xx[:, h * BLK:(h + 1) * BLK]
                        ar = ar + xh * wr_ref[:, cs]
                for c in range(0, D, 2 * BLK):
                    xx = x_v[r:r + 8, c:c + 2 * BLK].astype(f32)
                    for h in range(2):
                        cs = slice(c + h * BLK, c + (h + 1) * BLK)
                        xh = xx[:, h * BLK:(h + 1) * BLK]
                        ag = ag + xh * gw_ref[:, cs]
                prev = ar + ag
                accs[0].append(ar)
                accs[1].append(ag)
            sums = [jnp.sum(jnp.concatenate(a, axis=0).T, axis=0, keepdims=True) for a in accs]
            rows.append(sums[0])
            gate = jnp.broadcast_to(_sigmoid(sums[1]), (BLK, BLK)).T
            gate_v[t * BLK:(t + 1) * BLK, :] = gate
            ends.append(gate[BLK - 8:])
        r = jnp.concatenate(rows, axis=1).astype(bf16).astype(f32)
        r_max = jnp.max(r, axis=1, keepdims=True)
        lane = lax.broadcasted_iota(jnp.int32, (1, S), 1)
        idx_v = jnp.min(jnp.where(r == r_max, lane, S), axis=1, keepdims=True)
        idx_v = jnp.clip(idx_v, 0, S - 1)
        sel_v[0] = jnp.broadcast_to(_sigmoid(r_max), (8, BLK))
        sel_v[1] = jnp.broadcast_to(idx_v.astype(f32), (8, BLK))
        idx = idx_v[0, 0]
        state["idx"] = idx
        base = pl.multiple_of((idx // 16) * 16, 16)
        slab = x_v[pl.ds(base, 16), :].astype(f32)
        rid = lax.broadcasted_iota(jnp.int32, (16, D), 0)
        x_sel = jnp.sum(jnp.where(rid == idx - base, slab, 0.0), axis=0, keepdims=True)
        xc = jnp.broadcast_to(x_sel, (BLK, D)).T
        xc_v[...] = xc
        return last_slabs(xc) + _tree_sum(ends)

    def last_slabs(a):
        n = a.shape[0] // BLK
        return jnp.sum(a.reshape(n, BLK // 8, 8, BLK)[:, BLK // 8 - 1], axis=0)

    def b5():
        live = get_live()
        for f in (4, 3):
            free_forms(wk_v, wks_v, 0, HD, HD, f)
        z = k_epi(1, _strassen_tail2(k_prod(1), k_post, [ck_v[i] for i in range(4)]), None)
        z = k_epi(0, [_phi(c0_v[r:r + R, c:c + HD]) for r in (0, R) for c in (0, HD)], z)
        sep_forms(2, (2, 1, 0, 4, 3))
        z = k_epi(2, _strassen(k_prod(2), k_post), z)
        sep_forms(3, (2, 1, 0, 4, 3))
        z = k_epi(3, _strassen(k_prod(3), k_post), z)
        z = jnp.sum(z, axis=0, keepdims=True)
        zc = jnp.broadcast_to(z, (BLK, D)).T
        zc_v[...] = zc
        sep_forms(0, (4, 3, 0))
        end = router(live, _tree_sum(done) + last_slabs(zc))

        m3 = g_prod(2, R, HS - R) + g_prod(2, 0, R) + g_prod(2, HS - R, HS)
        order = G_ORDER
        m = {}
        for i in order:
            m[i] = g_prod2(i, i)
            if i == order[-1]:
                link = jnp.concatenate([_link(live, end)] * (HD // BLK), axis=1)
                m[i] = jnp.concatenate([m[i][:HD - 8], m[i][HD - 8:] + link], axis=0)
            if i == 4:
                g_v[0:HD // 2, HD:D] = _pk(m3 + m[4])
            if i in (1, 3) and 1 in m and 3 in m:
                g_v[HD // 2:D // 2, 0:HD] = _pk(m[1] + m[3])
        m1, m2, m4, m5 = m[0], m[1], m[3], m[4]
        cg_v[0] = m1 + (m4 - m5)
        cg_v[1] = m1 + (m3 - m2)

    def b6():
        live = get_live()
        sep_forms(0, (1, 2))
        g_v[0:HD // 2, 0:HD] = _pk(cg_v[0] + g_prod(6, R, HS) + g_prod(6, 0, R))
        g_v[HD // 2:D // 2, HD:D] = _pk(cg_v[1] + g_prod(5))
        end = make_wq_forms(live, 3)
        (gg, uu), end = _matvec_chain((v["wg_v"], v["wu_v"]), xc_v, D, F, live, 2 * BLK, end)
        gu_v[0] = gg
        gu_v[1] = uu
        head = _strassen_head(anchored(q_prod(0), 0, wqs_v, B_FORM[0], live, end), q_post)
        for i in range(4):
            cq_v[i] = head[i]

    def a_post(j):
        def post(a, col, half):
            rr = j * R + half * HS
            cs = slice(col * HD, (col + 1) * HD)
            g = jnp.tile(gate_v[rr:rr + R, :], (1, HD // BLK))
            b = x_v[rr:rr + R, cs].astype(f32)
            out_v[rr:rr + R, cs] = (b + g * (a - b)).astype(bf16)
            k = OUT_ORDER[col].index(rr)
            if k:
                start_out(col, k)
        return post

    def pair_post(j):
        def post(a, col, half):
            for n in range(2):
                a_post(j + n)(a[n * R:(n + 1) * R], col, half)
        return post

    def b7():
        live = get_live()
        sel_idx()
        gg = jnp.sum(gu_v[0], axis=0, keepdims=True)
        uu = jnp.sum(gu_v[1], axis=0, keepdims=True)
        hh = gg * _sigmoid(gg) * uu
        hc = jnp.broadcast_to(hh, (BLK, F)).T
        hc_v[...] = hc
        p = _strassen_tail(q_prod(0), q_post, [cq_v[i] for i in range(4)])
        ri = lax.broadcasted_iota(jnp.int32, (BLK, BLK), 0) // DH
        ci = lax.broadcasted_iota(jnp.int32, (BLK, BLK), 1) // DH
        diag = ri == ci
        kvs = []
        for j in range(NB):
            sl = slice(j * BLK, (j + 1) * BLK)
            kv = _dot(_unpk(g_v[j * BLK // 2:(j + 1) * BLK // 2, :]), v["wv_v"][:, sl])
            kvs.append(jnp.where(diag, kv, 0.0).astype(bf16))
        q_epi(0, p)
        for j in range(NB // 2):
            j2 = j + NB // 2
            mu = _dot(kvs[j], v["wo_v"][j * BLK:(j + 1) * BLK, :])
            ml = _dot(kvs[j2], v["wo_v"][j2 * BLK:(j2 + 1) * BLK, :])
            fs = _forms(mu[:, :HD], mu[:, HD:], ml[:, :HD], ml[:, HD:])
            for f in range(7):
                ms_v.put(fs[f], f, j * BLK)
        ends = [q_epi(1, _strassen(anchored(q_prod(1), 2, wqs_v, B_FORM[2], live, last_slabs(hc)),
                                   q_post)),
                q_epi(2, _strassen(q_prod(2), q_post)),
                q_epi(3, _strassen(q_prod(3), q_post))]
        prod = anchored(a_prod2(0), 1, ms_v, B_FORM[1], live, _tree_sum(ends))
        m3 = prod(2)
        m4 = prod(3)
        m5 = prod(4)
        pair_post(0)(m3 + m5, 1, 0)
        m2 = prod(1)
        pair_post(0)(m2 + m4, 0, 1)
        ck_v[0:2] = (m4 - m5).reshape(2, R, HD)
        ck_v[2:4] = (m3 - m2).reshape(2, R, HD)

    def b8():
        live = get_live()
        idx = sel_idx()
        (yy,), end = _matvec_chain((v["wd_v"],), hc_v, F, D, live, 2 * BLK, zero)
        y = jnp.sum(yy, axis=0, keepdims=True) * sel_v[0, 0:1, 0:1]

        prod = a_prod2(0)
        prod = anchored(prod, 5, ms_v, B_FORM[5], live, end)
        m1 = prod(0)
        _strassen_tail(prod, pair_post(0), (None, None, ck_v[0:2].reshape(2 * R, HD) + m1,
                                            ck_v[2:4].reshape(2 * R, HD) + m1))

        def patch():
            rid = lax.broadcasted_iota(jnp.int32, (16, HD), 0)
            for col in range(2):
                cs = slice(col * HD, (col + 1) * HD)
                base = jnp.where(idx % HS < N_LAG // 2 * R, (idx // 16) * 16, OUT_ORDER[col][N_LAG - 1])
                base = pl.multiple_of(base, 16)
                g = jnp.tile(gate_v[pl.ds(base, 16), :], (1, HD // BLK))
                upd = jnp.where(rid == idx - base, (1.0 - g) * y[:, cs], 0.0)
                out_v[pl.ds(base, 16), cs] = (out_v[pl.ds(base, 16), cs].astype(f32) + upd).astype(bf16)
                start_out(col, 0)
                base = pl.multiple_of((idx // 16) * 16, 16)
                upd = jnp.where(rid == idx - base, y[:, cs], 0.0)
                x_v[pl.ds(base, 16), cs] = (x_v[pl.ds(base, 16), cs].astype(f32) + upd).astype(bf16)

        def last_post(a, col, half):
            if (col, half) == (1, 0):
                patch()
            pair_post(2)(a, col, half)

        _strassen(a_prod2(2), last_post)

    return [ramp(i) for i in range(NK)] + [b4, b5, b6, b7, b8]


def _start_out(src, dst, sem, idx, col, k):
    order = OUT_ORDER[col]
    widths = [(col * HD, HD)]
    if k >= N_LAG:
        r0 = order[k]
        if col == 1 and k == len(order) - 1:
            widths = [(c, BLK) for c in range(HD, D, BLK)]
    else:
        blk = (idx // R) * R
        n = k if k else N_LAG - 1
        seen = functools.reduce(jnp.logical_or, [blk == r for r in order[:n]])
        r0 = jnp.where(seen, order[k], order[k - 1]) if k else jnp.where(seen, blk, order[N_LAG - 1])
        r0 = pl.multiple_of(r0, R)
    for c, n in widths:
        pltpu.make_async_copy(src.at[pl.ds(r0, R), pl.ds(c, n)], dst.at[pl.ds(r0, R), pl.ds(c, n)],
                              sem).start()


def _kernel(x_hbm, wqkv_hbm, wo_hbm, wr_hbm, wg_hbm, wu_hbm, wd_hbm, gw_hbm,
            out_hbm, *scratch):
    v = dict(zip(SCRATCH, scratch))
    sem_hi, sem_lo, sem_o = scratch[len(SCRATCH):]

    def x_copy(j, half):
        r0 = half * HS + j * R
        return pltpu.make_async_copy(x_hbm.at[0, pl.ds(r0, R), :], v["x_v"].at[pl.ds(r0, R), :],
                                     sem_hi.at[NK + min(j - 1, 1)])

    def ramp_copies(i):
        k0, n = K_CHUNKS[i]
        return [pltpu.make_async_copy(x_hbm.at[0, pl.ds(r0, R), pl.ds(k0, n)],
                                      v["x_v"].at[pl.ds(r0, R), pl.ds(k0, n)], sem_hi.at[i])
                for r0 in (0, HS)] + [
            pltpu.make_async_copy(wqkv_hbm.at[pl.ds(k0, n), pl.ds(D, D)],
                                  v["wk_v"].at[pl.ds(k0, n), :], sem_hi.at[i])]

    cp_wq = pltpu.make_async_copy(wqkv_hbm.at[:, pl.ds(0, D)], v["wq_v"], sem_lo.at[1])
    cp_wv = pltpu.make_async_copy(wqkv_hbm.at[:, pl.ds(2 * D, D)], v["wv_v"], sem_lo.at[2])
    cp_wo = pltpu.make_async_copy(wo_hbm, v["wo_v"], sem_lo.at[2])
    cp_wg = pltpu.make_async_copy(wg_hbm, v["wg_v"], sem_lo.at[1])
    cp_wu = pltpu.make_async_copy(wu_hbm, v["wu_v"], sem_lo.at[1])
    cp_wd = pltpu.make_async_copy(wd_hbm, v["wd_v"], sem_lo.at[3])
    cp_wr = pltpu.make_async_copy(wr_hbm, v["wr_v"], sem_lo.at[0])
    cp_gw = pltpu.make_async_copy(gw_hbm, v["gw_v"], sem_lo.at[0])

    state = {}

    waits = [ramp_copies(i) for i in range(NK)] + [
        [x_copy(1, 0), x_copy(1, 1)],
        [x_copy(j, h) for j in range(2, NP) for h in range(2)] + [cp_wr, cp_gw],
        [cp_wg, cp_wu, cp_wq],
        [cp_wv, cp_wo],
        [cp_wd],
    ]
    for cp in sum(waits[:NK + 1], []) + waits[NK + 1][:-2]:
        cp.start()
    blocks = _blocks(v, lambda col, k: _start_out(v["out_v"], out_hbm.at[0], sem_o, state["idx"], col, k),
                     state)
    for n, (ws, blk) in enumerate(zip(waits, blocks)):
        for cp in ws:
            cp.wait()
        if n == 3:
            for cp in (cp_wr, cp_gw, cp_wg, cp_wu, cp_wq, cp_wv, cp_wo, cp_wd):
                cp.start(priority=1)
        blk()
    pltpu.make_async_copy(v["out_v"], out_hbm.at[0], sem_o).wait()


@jax.jit
def pallas_gated_mix__linear_attn_block__moe_arch_mod__prompt_kernel(
    A_x: jax.Array,
    A_wqkv: jax.Array,
    A_wo: jax.Array,
    B_x: jax.Array,
    B_w_r: jax.Array,
    B_w_gate: jax.Array,
    B_w_up: jax.Array,
    B_w_down: jax.Array,
    gate_w: jax.Array,
):
    del B_x
    any_spec = pl.BlockSpec(memory_space=pl.ANY)
    scratch = [pltpu.VMEM(*s) for s in SCRATCH.values()] + [
        pltpu.SemaphoreType.DMA((NK + 2,)),
        pltpu.SemaphoreType.DMA((4,)),
        pltpu.SemaphoreType.DMA(()),
    ]
    return pl.pallas_call(
        _kernel,
        out_shape=jax.ShapeDtypeStruct((1, S, D), bf16),
        in_specs=[any_spec] * 8,
        out_specs=any_spec,
        scratch_shapes=scratch,
        compiler_params=pltpu.CompilerParams(vmem_limit_bytes=120 * 1024 * 1024,
                                             disable_semaphore_checks=True),
    )(A_x, A_wqkv, A_wo, B_w_r, B_w_gate, B_w_up, B_w_down, gate_w)
```
